```python
import os as _os
_os.environ.setdefault("JAX_PLATFORMS", "cpu")
import jax
import jax.numpy as jnp

def _softmax(x, axis=-1):
    return jax.nn.softmax(x, axis=axis)
def _gelu(x):
    return jax.nn.gelu(x, approximate=True)
def _silu(x):
    return jax.nn.silu(x)
def _sigmoid(x):
    return jax.nn.sigmoid(x)
def _layernorm(x, axis=-1, eps=1e-5):
    m = jnp.mean(x, axis=axis, keepdims=True)
    v = jnp.var(x, axis=axis, keepdims=True)
    return (x - m) / jnp.sqrt(v + eps)
def _scatter_add(tgt, idx, src, axis=0):
    return tgt.at[idx].add(src)
def _segment_sum(src, seg, n):
    return jax.ops.segment_sum(src, seg, n)
class _Rng:
    def __init__(self, key):
        self._k = key
    def _next(self):
        self._k, sub = jax.random.split(self._k)
        return sub
    def normal(self, shape):
        return jax.random.normal(self._next(), shape, dtype=jnp.bfloat16)
    def randint(self, lo, hi, shape):
        return jax.random.randint(self._next(), shape, lo, hi, dtype=jnp.int32)
    def uniform(self, shape, lo=0.0, hi=1.0):
        return jax.random.uniform(self._next(), shape, jnp.bfloat16, lo, hi)
    def permutation(self, n):
        return jax.random.permutation(self._next(), n)


kernel_name = 'concat_heads__sliding_block__ssm_conv_s4__prompt'

def setup_inputs():
    _rng = _Rng(jax.random.key(int.from_bytes(__import__("os").urandom(4), "little")))
    _w = (lambda a: (lambda t: t.astype(jnp.bfloat16) if jnp.issubdtype(t.dtype, jnp.floating) else t)(jnp.asarray(a)))
    def _A_setup():
        B, S, D = 1, 2048, 512
        return {
            "x": _w((lambda *s: _rng.normal(s) * 0.2)(B, S, D)),
            "wqkv": _w((lambda *s: _rng.normal(s) * 0.2)(D, 3 * D)),
            "wo": _w((lambda *s: _rng.normal(s) * 0.05)(D, D)),
        }
    _A_in = _A_setup()

    def _B_setup():
        B, L, D, N = 1, 2048, 512, 128
        A_re = -jnp.exp((lambda *s: _rng.normal(s) * 0.8)(D, N))
        A_im = jnp.pi * (lambda *s: _rng.normal(s) * 0.8)(D, N)
        B_re = (lambda *s: _rng.normal(s) * 0.8)(D, N)
        B_im = (lambda *s: _rng.normal(s) * 0.8)(D, N)
        C_re = (lambda *s: _rng.normal(s) * 0.8)(D, N)
        C_im = (lambda *s: _rng.normal(s) * 0.8)(D, N)
        log_dt = (lambda *s: _rng.normal(s) * 0.8)(D) * 0.5 - 4.0
        Dskip = (lambda *s: _rng.normal(s) * 0.05)(D)
        return {
            "u": _w((lambda *s: _rng.normal(s) * 0.05)(B, L, D)),
            "A_re": _w(A_re),
            "A_im": _w(A_im),
            "B_re": _w(B_re),
            "B_im": _w(B_im),
            "C_re": _w(C_re),
            "C_im": _w(C_im),
            "log_dt": _w(log_dt),
            "Dskip": _w(Dskip),
        }
    _B_in = _B_setup()

    return {
        "A_x": _A_in["x"],
        "A_wqkv": _A_in["wqkv"],
        "A_wo": _A_in["wo"],
        "B_u": _B_in["u"],
        "B_A_re": _B_in["A_re"],
        "B_A_im": _B_in["A_im"],
        "B_B_re": _B_in["B_re"],
        "B_B_im": _B_in["B_im"],
        "B_C_re": _B_in["C_re"],
        "B_C_im": _B_in["C_im"],
        "B_log_dt": _B_in["log_dt"],
        "B_Dskip": _B_in["Dskip"],
    }

def reference(A_x, A_wqkv, A_wo, B_u, B_A_re, B_A_im, B_B_re, B_B_im, B_C_re, B_C_im, B_log_dt, B_Dskip):
    def _A_ref(x, wqkv, wo):
        B, S, D = x.shape
        H = 32; Dh = D // H; W = 256
        qkv = (lambda x, *d: x.transpose(*d))((x @ wqkv).reshape(B, S, 3, H, Dh), 2, 0, 3, 1, 4)
        q, k, v = qkv[0], qkv[1], qkv[2]
        scores = jnp.einsum("bhqd,bhkd->bhqk", q, k) * (Dh ** -0.5)
        idx = jnp.arange(S)
        mask = (idx[:, None] - idx[None, :] >= 0) & (idx[:, None] - idx[None, :] < W)
        scores = jnp.where(mask[None, None], scores, -1e9)
        p = _softmax(scores, axis=-1)
        o = jnp.einsum("bhqk,bhkd->bhqd", p, v)
        return (lambda x, *d: x.transpose(*d))(o, 0, 2, 1, 3).reshape(B, S, D) @ wo

    def _B_ref(u, A_re, A_im, B_re, B_im, C_re, C_im, log_dt, Dskip):
        Bsz, L, D = u.shape
        dt = jnp.exp(log_dt)[:, None]
        A = A_re + 1j * A_im
        Bc = B_re + 1j * B_im
        Cc = C_re + 1j * C_im
        logdA = dt * A
        dB = dt * Bc
        l = (lambda x, dt: x.astype(dt))(jnp.arange(L), A_re.dtype)
        P = jnp.exp(logdA[:, :, None] * l[None, None, :])
        K = jnp.einsum("dn,dnl,dn->dl", Cc, P, dB).real
        L2 = 2 * L
        Kp = jnp.pad(K, ((0, 0), (0, L)))
        up = (lambda x, *d: x.transpose(*d))(u, 0, 2, 1)
        up = jnp.pad(up, ((0, 0), (0, 0), (0, L)))
        Kf = (lambda x, axes=(-2,-1): jnp.fft.rfft2(x.astype(jnp.float32), axes=axes))(Kp[:, None, :], axes=(-2, -1))
        Uf = (lambda x, axes=(-2,-1): jnp.fft.rfft2(x.astype(jnp.float32), axes=axes))(up[:, :, None, :], axes=(-2, -1))
        Yf = Uf * Kf[None, :, :, :]
        y = (lambda x, s, axes=(-2,-1): jnp.fft.irfft2(x, s=s, axes=axes).astype(jnp.bfloat16))(Yf, (1, L2), axes=(-2, -1))[:, :, 0, :L]
        y = (lambda x, *d: x.transpose(*d))(y, 0, 2, 1) + u * Dskip[None, None, :]
        return y

    a = _A_ref(A_x, A_wqkv, A_wo)
    b = _B_ref(B_u, B_A_re, B_A_im, B_B_re, B_B_im, B_C_re, B_C_im, B_log_dt, B_Dskip)
    return jnp.concatenate([a, b], axis=-1)
```

```python
import math

import jax
import jax.numpy as jnp
from jax import lax
import jax.experimental.pallas as pl
import jax.experimental.pallas.tpu as pltpu

F32 = jnp.float32
BF16 = jnp.bfloat16
I32 = jnp.int32
NT = (((1,), (1,)), ((), ()))

SEQ = 2048
DM = 512
QSCALE = 0.25 * math.log2(math.e)
NEG = -1e30

UP = 33
HP = 33
SPB = 72
YP = 72
VP = 9
TB = 256
UNR_PREP = 4
UNR_GE = 4


def bc16(x):
    return pltpu.bitcast(x, BF16)


def bc32(x):
    return pltpu.bitcast(x, I32)


def pk(lo, hi):
    return pltpu.pack_elementwise([lo, hi], packed_dtype=BF16)


def lo16(w):
    return pltpu.bitcast(w << 16, F32)


def hi16(w):
    return pltpu.bitcast(w & (-0x10000), F32)


def cmul(ar, ai, br, bi):
    return ar * br - ai * bi, ar * bi + ai * br


def ldb(ref, *idx):
    *lead, r0, n = idx
    if isinstance(r0, int):
        s = pl.ds(r0 // 2, n // 2)
    else:
        s = pl.ds(pl.multiple_of(r0 // 2, 8), n // 2)
    return bc16(ref.bitcast(I32)[(*lead, s, slice(None))])


def prep_dt(logdt_ref, dtb):
    ld = logdt_ref[...].astype(F32).reshape(4, 128)
    dt = jnp.exp(ld).astype(BF16).astype(F32)
    for g in range(4):
        dtb[128 * g:128 * g + 128, :] = jnp.broadcast_to(dt[g:g + 1, :], (128, 128)).T


def csqrt(a, b):
    aa = jnp.abs(a)
    ab = jnp.abs(b)
    m = jnp.maximum(aa, ab)
    z = m == 0.0
    ms = jnp.where(z, 1.0, m)
    inv = 1.0 / ms
    an = aa * inv
    bn = ab * inv
    r = jnp.sqrt(an * an + bn * bn)
    tn = jnp.sqrt((r + an) * 0.5)
    tn = jnp.where(z, 1.0, tn)
    sm = jnp.sqrt(ms)
    t = tn * sm
    o = (bn / (2.0 * tn)) * sm
    sgn = jnp.where(b < 0, -1.0, 1.0)
    pos = a >= 0
    sr = jnp.where(pos, t, o)
    si = jnp.where(pos, o, t) * sgn
    return jnp.where(z, 0.0, sr), jnp.where(z, 0.0, si)


def prep_hex(params, tabs, h):
    Are, Aim, Bre, Bim, Cre, Cim = params
    dtb, V0r, V0i, P1r, P1i, P16r, P16i, P32r, P32i, Lr, Li, Qr, Qi, Wr = tabs
    rs = pl.ds(pl.multiple_of(h * 16, 16), 16)
    ld = lambda R: ldb(R, h * 16, 16).astype(F32)
    d = dtb[rs, :]
    zr = d * ld(Are)
    zi = d * ld(Aim)
    mag = jnp.exp(zr)
    e1r = mag * jnp.cos(zi)
    e1i = mag * jnp.sin(zi)
    wr, wi = cmul(ld(Cre), ld(Cim), d * ld(Bre), d * ld(Bim))
    w1r, w1i = cmul(wr, wi, e1r, e1i)
    sr, si = csqrt(w1r, w1i)
    Wr[rs, :] = wr
    Qr[rs, :] = sr
    Qi[rs, :] = si
    p2 = cmul(e1r, e1i, e1r, e1i)
    p4 = cmul(*p2, *p2)
    p8 = cmul(*p4, *p4)
    p16 = cmul(*p8, *p8)
    p32 = cmul(*p16, *p16)
    p64 = cmul(*p32, *p32)
    q0 = (sr, si)
    q1 = cmul(*q0, *p2)
    q2 = cmul(*q0, *p4)
    q3 = cmul(*q1, *p4)
    Q = [q0, q1, q2, q3] + [cmul(*q, *p8) for q in (q0, q1, q2, q3)]
    for j in range(8):
        for half in range(2):
            st = pl.ds(h * (16 * VP) + half * 8 * VP + j, 8, stride=VP)
            V0r[st, :] = Q[j][0][8 * half:8 * half + 8]
            V0i[st, :] = Q[j][1][8 * half:8 * half + 8]
    P1r[rs, :] = e1r
    P1i[rs, :] = e1i
    P16r[rs, :] = p16[0]
    P16i[rs, :] = p16[1]
    P32r[rs, :] = p32[0]
    P32i[rs, :] = p32[1]
    Lr[rs, :] = p64[0]
    Li[rs, :] = p64[1]


def dyn0(v):
    return v // 64


def lane_consts():
    l = lax.broadcasted_iota(I32, (8, 128), 1)
    m = jnp.where(l < 64, 0x0000FFFF, -0x10000).astype(I32)
    return l, m


def uprep(u_s, UE, g, j):
    l, m = lane_consts()
    T = bc32(ldb(u_s, g, j * 128, 128).T)
    for k in range(8):
        v = T[8 * k:8 * k + 8]
        A = jnp.take_along_axis(v, l ^ 63, axis=1, mode="promise_in_bounds") & m
        B = jnp.take_along_axis(v, 127 - l, axis=1, mode="promise_in_bounds") & m
        p0 = 64 * g + 8 * k
        UE[pl.ds(p0 * UP + 2 * j, 8, stride=UP), :] = A
        UE[pl.ds(p0 * UP + 2 * j + 1, 8, stride=UP), :] = B


def ggen(tabs, hx, c):
    dtb, V0r, V0i, P1r, P1i, P16r, P16i, P32r, P32i, Lr, Li, Qr, Qi, Wr = tabs
    d = hx * 16 + c
    ve = (V0r[pl.ds(d * VP, 8), :], V0i[pl.ds(d * VP, 8), :])
    row = lambda R: R[pl.ds(d, 1), :]
    p1 = (row(P1r), row(P1i))
    p16 = (row(P16r), row(P16i))
    p32 = (row(P32r), row(P32i))
    vo = cmul(*ve, *p1)
    V = [(ve, vo), (cmul(*ve, *p16), cmul(*vo, *p16))]
    V = V + [(cmul(*e, *p32), cmul(*o, *p32)) for e, o in V]
    return [pk(e[0], o[0]) for e, o in V], [pk(e[1], o[1]) for e, o in V]


def st_GE(tabs, UE, Gs, Sr, Si, hx):
    for pl_ in range(8):
        p = hx * 8 + pl_
        r1, i1 = ggen(tabs, hx, 2 * pl_)
        r2, i2 = ggen(tabs, hx, 2 * pl_ + 1)
        Gr = jnp.concatenate(r1 + r2, axis=0)
        Gi = jnp.concatenate(i1 + i2, axis=0)
        Gs[pl.ds(pl.multiple_of(p * 128, 128), 64), :] = Gr
        Gs[pl.ds(pl.multiple_of(p * 128 + 64, 64), 64), :] = Gi
        L = bc16(UE[pl.ds(p * UP, 32), :])
        rows = pl.ds(pl.multiple_of(p * SPB, 8), 64)
        Sr[rows, :] = jnp.dot(L, bc16(Gr), preferred_element_type=F32).astype(BF16)
        Si[rows, :] = jnp.dot(L, bc16(Gi), preferred_element_type=F32).astype(BF16)


def st_scan(tabs, Sr, Si, Hr, Hn, hx):
    dtb, V0r, V0i, P1r, P1i, P16r, P16i, P32r, P32i, Lr, Li, Qr, Qi, Wr = tabs
    base = hx * (8 * HP)
    W = SPB // 2
    Sv = [R.bitcast(I32).at[pl.ds(pl.multiple_of(hx * (8 * W), 4), 8 * W)] for R in (Sr, Si)]
    lam, first = [], []
    for ch in range(2):
        sl = pl.ds(hx * 16 + ch, 8, stride=2)
        lam.append((Lr[sl, :], Li[sl, :]))
        first.append((Qr[sl, :], -Qi[sl, :]))
    wst = lambda s_: pl.ds(base + s_, 8, stride=HP)

    def step(ch, sr, si, st):
        if st is None:
            return sr, -si
        H, N = st
        lr, li = lam[ch]
        return (lr * H + sr) + li * N, (lr * N - si) - li * H

    e0, o0 = first
    st0 = st1 = None
    for j in range(16):
        wa = [V[pl.ds(2 * j, 8, stride=W), :] for V in Sv]
        wb = [V[pl.ds(2 * j + 1, 8, stride=W), :] for V in Sv]
        st0 = step(0, lo16(wa[0]), lo16(wa[1]), st0)
        st1 = step(1, hi16(wb[0]), hi16(wb[1]), st1)
        e1, o1 = st0, st1
        Hr[wst(2 * j), :] = pk(e0[0], o1[0])
        Hn[wst(2 * j), :] = pk(e0[1], o1[1])
        Hr[wst(2 * j + 1), :] = pk(e1[0], o0[0])
        Hn[wst(2 * j + 1), :] = pk(e1[1], o0[1])
        if j < 15:
            st0 = step(0, lo16(wb[0]), lo16(wb[1]), st0)
            st1 = step(1, hi16(wa[0]), hi16(wa[1]), st1)
            e0, o0 = st0, st1


def st_F(Gs, Hr, Hn, Y1s, hx):
    for pl_ in range(8):
        p = hx * 8 + pl_
        rows = pl.ds(p * HP, 32)
        hr = bc16(Hr[rows, :])
        hn = bc16(Hn[rows, :])
        Gr = bc16(Gs[pl.ds(pl.multiple_of(p * 128, 128), 64), :])
        Gi = bc16(Gs[pl.ds(pl.multiple_of(p * 128 + 64, 64), 64), :])
        Y1s[pl_] = (lax.dot_general(hr, Gr, NT, preferred_element_type=F32)
                    + lax.dot_general(hn, Gi, NT, preferred_element_type=F32))


def st_T(UE, Y1s, YT, hx):
    l8 = lax.broadcasted_iota(I32, (8, 128), 1)
    r8 = lax.broadcasted_iota(I32, (8, 128), 0)
    rev = 7 - r8
    for pl_ in range(8):
        p = hx * 8 + pl_
        top = Y1s[pl_, 0:8, :]
        K1 = jnp.where(l8 < 64, jnp.broadcast_to(top[0:1], (8, 128)), 0.0)
        K2 = jnp.where(l8 >= 64, jnp.broadcast_to(top[3:4], (8, 128)), 0.0)
        tiles = []
        for K in (K1, K2):
            Kp = pk(pltpu.roll(K, 1, 1), K)
            for i in range(4):
                R = pltpu.roll(Kp, 49 - 16 * i, 1, stride=2, stride_axis=0)
                tiles.append(jnp.take_along_axis(R, rev, axis=0, mode="promise_in_bounds"))
        TK = bc16(jnp.concatenate(tiles, axis=0))
        L = bc16(UE[pl.ds(p * UP, 32), :])
        Y2 = jnp.dot(L, TK, preferred_element_type=F32)
        top = jnp.where((r8 == 0) | (r8 == 3), 0.0, top)
        Y = jnp.concatenate([top, Y1s[pl_, 8:64, :]], axis=0) + Y2
        YT[pl.ds(pl.multiple_of(p * YP, 8), 64), :] = Y.astype(BF16)


def ypost(YT, u_s, Dv, b_s, g, jj, e):
    l, m = lane_consts()
    W = YP // 2
    Yv = YT.bitcast(I32).at[pl.ds(pl.multiple_of(g * (64 * W) + 4 * jj, 4), 64 * W - 28)]
    A = jnp.concatenate([Yv[pl.ds(8 * k * W + 2 * e, 8, stride=W), :] for k in range(8)], axis=0)
    B = jnp.concatenate([Yv[pl.ds(8 * k * W + 2 * e + 1, 8, stride=W), :] for k in range(8)], axis=0)
    m64 = jnp.concatenate([m] * 8, axis=0)
    T = (A & m64) | (pltpu.roll(B, 64, 1) & (~m64))
    y = bc16(T).T
    j = 2 * jj + e
    u = ldb(u_s, g, j * 128, 128).astype(F32)
    b_s[g, pl.ds(pl.multiple_of(j * 128, 128), 128), :] = (
        y.astype(F32) + u * Dv[pl.ds(g, 1), :]).astype(BF16)


def wt_prep(w_s, wt_s):
    for c in range(4):
        for i, n in enumerate((0, 1, 2, 3, 8, 9, 10, 11)):
            wt_s[c, 128 * i:128 * i + 128, :] = ldb(w_s, n, 128 * c, 128).T


def proj_step(x_s, w_s, wt_s, k_s, qT_s, vT_s, j):
    t0 = pl.multiple_of(j * TB, TB)
    X = jnp.concatenate([ldb(x_s, c, t0, TB) for c in range(4)], axis=1)
    Wk = jnp.concatenate([ldb(w_s, 4 + g, 0, 512) for g in range(4)], axis=1)
    Kf = jnp.dot(X, Wk, preferred_element_type=F32)
    for g in range(4):
        k_s[g, pl.ds(t0, TB), :] = Kf[:, 128 * g:128 * g + 128].astype(BF16)
    WT = jnp.concatenate([ldb(wt_s, c, 0, 1024) for c in range(4)], axis=1)
    QV = lax.dot_general(WT, X, NT, preferred_element_type=F32)
    for b in range(TB // 128):
        i = j * (TB // 128) + b
        qT_s[i] = (QV[:512, 128 * b:128 * b + 128] * QSCALE).astype(BF16)
        vT_s[i] = QV[512:, 128 * b:128 * b + 128].astype(BF16)


def wq_tile(qT_s, i, g, h):
    qh = ldb(qT_s, i, (g * 8 + h) * 16, 16)
    parts = []
    if h > 0:
        parts.append(jnp.zeros((16 * h, 128), BF16))
    parts.append(qh)
    if h < 7:
        parts.append(jnp.zeros((16 * (7 - h), 128), BF16))
    return jnp.concatenate(parts, axis=0)


def stage_A(i, g, h0, kind, k_s, qT_s, sw, sy, sm, slot):
    r0 = i * 128
    Wq = jnp.concatenate([wq_tile(qT_s, i, g, h0 + a) for a in range(4)], axis=1)
    parts = []
    if kind == 2:
        for t in range(8):
            parts.append(ldb(k_s, g, r0 - 256 + 16 * t, 16))
            parts.append(ldb(k_s, g, r0 + 16 * t, 16))
        parts.append(ldb(k_s, g, r0 - 128, 128))
    else:
        parts.append(ldb(k_s, g, r0, 128))
        if kind == 1:
            parts.append(ldb(k_s, g, r0 - 128, 128))
    S = jnp.dot(jnp.concatenate(parts, axis=0), Wq, preferred_element_type=F32)
    rows = lax.broadcasted_iota(I32, (16, 128), 0)
    lanes = lax.broadcasted_iota(I32, (16, 128), 1)
    for a in range(4):
        Sa = S[:, a * 128:(a + 1) * 128]
        m = None
        for t in range(8):
            if kind == 2:
                X = Sa[32 * t:32 * t + 16]
                Z = Sa[32 * t + 16:32 * t + 32]
            else:
                X = jnp.full((16, 128), NEG, F32)
                Z = Sa[16 * t:16 * t + 16]
            W = jnp.where(rows + 16 * t <= lanes, Z, X)
            sw[slot, a, 16 * t:16 * t + 16, :] = W
            mm = jnp.maximum(W[:8], W[8:])
            m = mm if m is None else jnp.maximum(m, mm)
        if kind >= 1:
            Y = Sa[256:] if kind == 2 else Sa[128:]
            sy[slot, a] = Y
            for t in range(16):
                m = jnp.maximum(m, Y[8 * t:8 * t + 8])
        sm[slot, a] = m


def stage_B(i, g, h0, kind, vT_s, oT_s, sw, sy, sm, slot, oslot):
    lanes = lax.broadcasted_iota(I32, (128, 128), 1)
    rows = lax.broadcasted_iota(I32, (128, 128), 0)
    tri = rows <= lanes
    for a in range(4):
        hh = g * 8 + h0 + a
        m = jnp.max(sm[slot, a], axis=0, keepdims=True)
        pW = jnp.exp2(sw[slot, a] - m)
        vt = lambda blk: ldb(vT_s, blk, hh * 16, 16)
        if kind == 0:
            l = jnp.sum(pW, axis=0, keepdims=True)
            P = pW.astype(BF16)
            Vt = vt(i)
        else:
            pY = jnp.exp2(sy[slot, a] - m)
            l = jnp.sum(pW + pY, axis=0, keepdims=True)
            if kind == 1:
                P = jnp.concatenate([pY, pW], axis=0).astype(BF16)
                Vt = jnp.concatenate([vt(i - 1), vt(i)], axis=1)
            else:
                z = jnp.zeros_like(pW)
                P = jnp.concatenate([jnp.where(tri, z, pW), pY, jnp.where(tri, pW, z)],
                                    axis=0).astype(BF16)
                Vt = jnp.concatenate([vt(i - 2), vt(i - 1), vt(i)], axis=1)
        O = jnp.dot(Vt, P, preferred_element_type=F32) * (1.0 / l)
        oT_s[oslot, hh * 16:(hh + 1) * 16, :] = O.astype(BF16)


def outproj(oT_s, oslot, wo_s, a_s, i):
    O = jnp.concatenate([ldb(oT_s, oslot, 128 * c, 128).T for c in range(4)], axis=1)
    Wo = jnp.concatenate([ldb(wo_s, n, 0, 512) for n in range(4)], axis=1)
    A = jnp.dot(O, Wo, preferred_element_type=F32)
    r = pl.ds(pl.multiple_of(i * 128, 128), 128)
    for n in range(4):
        a_s[n, r, :] = A[:, 128 * n:128 * n + 128].astype(BF16)


def kernel_body(x_h, w_h, wo_h, u_h, Are_h, Aim_h, Bre_h, Bim_h, Cre_h, Cim_h, ldt_h, D_h,
                out_h,
                x_s, w_s, wo_s, u_s, Are, Aim, Bre, Bim, Cre, Cim, ldt_v, D_v,
                a_s, b_s, sems,
                wt_s, k_s, qT_s, vT_s, oT_s, sw, sy, sm, Dv, *scr):
    tabs = scr[:14]
    UE, Gs, Sr, Si, Hr, Hn, Y1e, Y1o, YT = scr[14:]
    z = pl.program_id(0)

    cp_par = [pltpu.make_async_copy(s, d, sems.at[0]) for s, d in (
        (ldt_h, ldt_v), (D_h, D_v), (Are_h, Are), (Aim_h, Aim), (Bre_h, Bre),
        (Bim_h, Bim), (Cre_h, Cre), (Cim_h, Cim))]
    cp_u = [pltpu.make_async_copy(u_h.at[0, :, pl.ds(128 * g, 128)], u_s.at[g], sems.at[1 + g])
            for g in range(4)]
    cp_x = [pltpu.make_async_copy(x_h.at[0, :, pl.ds(128 * c, 128)], x_s.at[c], sems.at[5])
            for c in range(4)]
    cp_w = [pltpu.make_async_copy(w_h.at[:, pl.ds(128 * n, 128)], w_s.at[n], sems.at[6])
            for n in range(12)]
    cp_wo = [pltpu.make_async_copy(wo_h.at[:, pl.ds(128 * n, 128)], wo_s.at[n], sems.at[7])
             for n in range(4)]
    for c in cp_par + cp_u + cp_w + cp_x + cp_wo:
        c.start()

    def a_copy(i, n):
        r = pl.ds(pl.multiple_of(i * 128, 128), 128)
        return pltpu.make_async_copy(a_s.at[n, r, :], out_h.at[0, r, pl.ds(128 * n, 128)], sems.at[8])

    def b_copy(g):
        return pltpu.make_async_copy(b_s.at[g], out_h.at[0, :, pl.ds(DM + 128 * g, 128)], sems.at[9])

    for c in cp_par:
        c.wait()
    prep_dt(ldt_v, tabs[0])
    params = (Are, Aim, Bre, Bim, Cre, Cim)
    for g in range(4):
        cp_u[g].wait()

        @pl.loop(0, 8 // UNR_PREP)
        def _(hh):
            for i in range(UNR_PREP):
                prep_hex(params, tabs, 8 * g + hh * UNR_PREP + i)
            for i in range(2 * UNR_PREP):
                uprep(u_s, UE, g, hh * (2 * UNR_PREP) + i)

    Wr = tabs[13]
    Dv[0:4, :] = D_v[...].astype(F32).reshape(4, 128) + jnp.concatenate(
        [jnp.sum(Wr[128 * g:128 * g + 128, :].T, axis=0, keepdims=True) for g in range(4)], axis=0)

    @pl.loop(0, 32 // UNR_GE)
    def _(q):
        for i in range(UNR_GE):
            st_GE(tabs, UE, Gs, Sr, Si, UNR_GE * q + i)

    for c in cp_w:
        c.wait()
    wt_prep(w_s, wt_s)
    for c in cp_x:
        c.wait()
    nstep = SEQ // TB
    hps = 32 // nstep

    @pl.loop(0, nstep)
    def _(j):
        proj_step(x_s, w_s, wt_s, k_s, qT_s, vT_s, j)
        for i in range(hps):
            st_scan(tabs, Sr, Si, Hr, Hn, j * hps + i)

    st_F(Gs, Hr, Hn, Y1e, z)

    @pl.loop(0, 15)
    def _(q):
        st_F(Gs, Hr, Hn, Y1o, 2 * q + 1)
        st_T(UE, Y1e, YT, 2 * q)
        st_F(Gs, Hr, Hn, Y1e, 2 * q + 2)
        st_T(UE, Y1o, YT, 2 * q + 1)

    st_F(Gs, Hr, Hn, Y1o, z + 31)
    st_T(UE, Y1e, YT, z + 30)
    st_T(UE, Y1o, YT, z + 31)

    for c in cp_wo:
        c.wait()
    steps = [(g, h0) for g in range(4) for h0 in (0, 4)]
    A = lambda i, s, kind, slot: stage_A(i, *steps[s], kind, k_s, qT_s, sw, sy, sm, slot)
    B = lambda i, s, kind, slot, osl: stage_B(i, *steps[s], kind, vT_s, oT_s, sw, sy, sm, slot, osl)

    def yp(i, s):
        if s in (0, 2, 4, 6):
            c = s // 2
            ypost(YT, u_s, Dv, b_s, i // 4, 2 * (i % 4) + c // 2, c % 2)

    def start_out(i):
        for n in range(4):
            a_copy(i, n).start()

    A(0, 0, 0, 0)
    for s in range(8):
        if s < 7:
            A(0, s + 1, 0, (s + 1) % 2)
        else:
            A(1, 0, 1, 0)
        B(0, s, 0, s % 2, 0)
        yp(z, s)
    for s in range(8):
        if s < 7:
            A(1, s + 1, 1, (s + 1) % 2)
        else:
            A(2, 0, 2, 0)
        B(1, s, 1, s % 2, 1)
        yp(z + 1, s)
        if s == 1:
            outproj(oT_s, 0, wo_s, a_s, 0)
        if s == 5:
            start_out(z)

    @pl.loop(1, 8)
    def _(ii):
        for e in range(2):
            i = 2 * ii + e
            for s in range(8):
                if s < 7:
                    A(i, s + 1, 2, (s + 1) % 2)
                else:
                    A(jnp.minimum(i + 1, 15), 0, 2, 0)
                B(i, s, 2, s % 2, e)
                yp(i, s)
                if s == 1:
                    outproj(oT_s, 1 - e, wo_s, a_s, i - 1)
                if s == 5:
                    start_out(i - 1)

        @pl.when(ii % 2 == 1)
        def _():
            b_copy(ii // 2).start()

    outproj(oT_s, 1, wo_s, a_s, z + 15)
    start_out(z + 15)
    for g in range(4):
        b_copy(g).wait()

    @pl.loop(0, 16)
    def _(i):
        for n in range(4):
            a_copy(i, n).wait()


def _scratch():
    T = lambda r: pltpu.VMEM((r, 128), F32)
    V = pltpu.VMEM
    s = [V((4, SEQ, 128), BF16), V((12, DM, 128), BF16), V((4, DM, 128), BF16), V((4, SEQ, 128), BF16)]
    s += [V((DM, 128), BF16)] * 6 + [V((DM,), BF16)] * 2
    s += [V((4, SEQ, 128), BF16), V((4, SEQ, 128), BF16), pltpu.SemaphoreType.DMA((10,))]
    s += [V((4, 1024, 128), BF16), V((4, SEQ, 128), BF16), V((16, DM, 128), BF16), V((16, DM, 128), BF16),
          V((2, DM, 128), BF16), V((2, 4, 128, 128), F32), V((2, 4, 128, 128), F32), V((2, 4, 8, 128), F32),
          T(8)]
    s += [T(512), T(512 * VP), T(512 * VP)] + [T(512)] * 11
    s += [V((256 * UP, 128), I32), V((256 * 128, 128), I32),
          V((256 * SPB, 128), BF16), V((256 * SPB, 128), BF16),
          V((256 * HP, 128), I32), V((256 * HP, 128), I32),
          V((8, 64, 128), F32), V((8, 64, 128), F32), V((256 * YP, 128), BF16)]
    return s


@jax.jit
def pallas_concat_heads__sliding_block__ssm_conv_s4__prompt_kernel(
    A_x: jax.Array,
    A_wqkv: jax.Array,
    A_wo: jax.Array,
    B_u: jax.Array,
    B_A_re: jax.Array,
    B_A_im: jax.Array,
    B_B_re: jax.Array,
    B_B_im: jax.Array,
    B_C_re: jax.Array,
    B_C_im: jax.Array,
    B_log_dt: jax.Array,
    B_Dskip: jax.Array,
):
    hbm = pl.BlockSpec(memory_space=pl.ANY)
    return pl.pallas_call(
        kernel_body,
        grid=(1,),
        in_specs=[hbm] * 12,
        out_specs=hbm,
        out_shape=jax.ShapeDtypeStruct((1, SEQ, 2 * DM), BF16),
        scratch_shapes=_scratch(),
        compiler_params=pltpu.CompilerParams(vmem_limit_bytes=110 * 1024 * 1024),
    )(A_x, A_wqkv, A_wo, B_u, B_A_re, B_A_im, B_B_re, B_B_im, B_C_re, B_C_im, B_log_dt, B_Dskip)
```

```python
import math

import jax
import jax.numpy as jnp
from jax import lax
import jax.experimental.pallas as pl
import jax.experimental.pallas.tpu as pltpu

F32 = jnp.float32
BF16 = jnp.bfloat16
I32 = jnp.int32
NT = (((1,), (1,)), ((), ()))

SEQ = 2048
DM = 512
QSCALE = 0.25 * math.log2(math.e)
NEG = -1e30

UP = 33
HP = 33
SPB = 72
YP = 72
VP = 9
TB = 256
UNR_FT = 16
NP = (16, 24, 32)
UNR_Q2 = 2
KC = 64
UNR_GE = 16


def bc16(x):
    return pltpu.bitcast(x, BF16)


def bc32(x):
    return pltpu.bitcast(x, I32)


def pk(lo, hi):
    return pltpu.pack_elementwise([lo, hi], packed_dtype=BF16)


def lo16(w):
    return pltpu.bitcast(w << 16, F32)


def hi16(w):
    return pltpu.bitcast(w & (-0x10000), F32)


def cmul(ar, ai, br, bi):
    return ar * br - ai * bi, ar * bi + ai * br


def ldb(ref, *idx):
    *lead, r0, n = idx
    if isinstance(r0, int):
        s = pl.ds(r0 // 2, n // 2)
    else:
        s = pl.ds(pl.multiple_of(r0 >> 1, 8), n // 2)
    return bc16(ref.bitcast(I32)[(*lead, s, slice(None))])


def rows(ref, start, n, mult=None):
    if mult is not None:
        start = pl.multiple_of(start, mult)
    return ref.at[pl.ds(start, n)]


def prep_dt(logdt_ref, dtb):
    ld = logdt_ref[...].astype(F32).reshape(4, 128)
    dt = jnp.exp(ld).astype(BF16).astype(F32)
    for g in range(4):
        dtb[128 * g:128 * g + 128, :] = jnp.broadcast_to(dt[g:g + 1, :], (128, 128)).T


def csqrt(a, b):
    aa = jnp.abs(a)
    ab = jnp.abs(b)
    m = jnp.maximum(aa, ab)
    z = m == 0.0
    ms = jnp.where(z, 1.0, m)
    inv = 1.0 / ms
    an = aa * inv
    bn = ab * inv
    r = jnp.sqrt(an * an + bn * bn)
    tn = jnp.sqrt((r + an) * 0.5)
    tn = jnp.where(z, 1.0, tn)
    sm = jnp.sqrt(ms)
    t = tn * sm
    o = (bn / (2.0 * tn)) * sm
    sgn = jnp.where(b < 0, -1.0, 1.0)
    pos = a >= 0
    sr = jnp.where(pos, t, o)
    si = jnp.where(pos, o, t) * sgn
    return jnp.where(z, 0.0, sr), jnp.where(z, 0.0, si)


def prep_hex(params, tabs, h):
    Are, Aim, Bre, Bim, Cre, Cim = params
    dtb, V0r, V0i, P1r, P1i, P16r, P16i, P32r, P32i, Lr, Li, Qr, Qi, Wr = tabs
    rs = pl.ds(pl.multiple_of(h * 16, 16), 16)
    ld = lambda R: ldb(R, h * 16, 16).astype(F32)
    d = dtb[rs, :]
    zr = d * ld(Are)
    zi = d * ld(Aim)
    mag = jnp.exp(zr)
    e1r = mag * jnp.cos(zi)
    e1i = mag * jnp.sin(zi)
    wr, wi = cmul(ld(Cre), ld(Cim), d * ld(Bre), d * ld(Bim))
    w1r, w1i = cmul(wr, wi, e1r, e1i)
    sr, si = csqrt(w1r, w1i)
    Wr[rs, :] = wr
    Qr[rs, :] = sr
    Qi[rs, :] = si
    p2 = cmul(e1r, e1i, e1r, e1i)
    p4 = cmul(*p2, *p2)
    p8 = cmul(*p4, *p4)
    p16 = cmul(*p8, *p8)
    p32 = cmul(*p16, *p16)
    p64 = cmul(*p32, *p32)
    q0 = (sr, si)
    q1 = cmul(*q0, *p2)
    q2 = cmul(*q0, *p4)
    q3 = cmul(*q1, *p4)
    Q = [q0, q1, q2, q3] + [cmul(*q, *p8) for q in (q0, q1, q2, q3)]
    V0rv, V0iv = rows(V0r, h * (16 * VP), 16 * VP), rows(V0i, h * (16 * VP), 16 * VP)
    for j in range(8):
        for half in range(2):
            st = pl.ds(half * 8 * VP + j, 8, stride=VP)
            V0rv[st, :] = Q[j][0][8 * half:8 * half + 8]
            V0iv[st, :] = Q[j][1][8 * half:8 * half + 8]
    P1r[rs, :] = e1r
    P1i[rs, :] = e1i
    P16r[rs, :] = p16[0]
    P16i[rs, :] = p16[1]
    P32r[rs, :] = p32[0]
    P32i[rs, :] = p32[1]
    Lr[rs, :] = p64[0]
    Li[rs, :] = p64[1]


def dyn0(v):
    return v // 64


def lane_consts():
    l = lax.broadcasted_iota(I32, (8, 128), 1)
    m = jnp.where(l < 64, 0x0000FFFF, -0x10000).astype(I32)
    return l, m


def uprep(u_s, UE, g, j):
    l, m = lane_consts()
    rev = 7 - lax.broadcasted_iota(I32, (8, 128), 0)
    U = u_s.bitcast(I32).at[g, pl.ds(pl.multiple_of(64 * j, 64), 64), :]
    parts = []
    for c in range(2):
        for v in range(4):
            w = jnp.take_along_axis(U[pl.ds(32 * c + 8 * (3 - v), 8), :], rev, axis=0, mode="promise_in_bounds")
            parts.append((w << 16) | lax.shift_right_logical(w, 16))
    T = bc32(bc16(jnp.concatenate(parts, axis=0)).T)
    UEv = rows(UE, 64 * UP * g + 2 * j, 63 * UP + 2)
    for k in range(8):
        v = T[8 * k:8 * k + 8]
        UEv[pl.ds(8 * k * UP, 8, stride=UP), :] = v & m
        UEv[pl.ds(8 * k * UP + 1, 8, stride=UP), :] = pltpu.roll(v, 64, 1) & m


def ggen(tv, c):
    V0r, V0i, P1r, P1i, P16r, P16i, P32r, P32i = tv
    ve = (V0r[pl.ds(c * VP, 8), :], V0i[pl.ds(c * VP, 8), :])
    row = lambda R: R[pl.ds(c, 1), :]
    p1 = (row(P1r), row(P1i))
    p16 = (row(P16r), row(P16i))
    p32 = (row(P32r), row(P32i))
    vo = cmul(*ve, *p1)
    V = [(ve, vo), (cmul(*ve, *p16), cmul(*vo, *p16))]
    V = V + [(cmul(*e, *p32), cmul(*o, *p32)) for e, o in V]
    return [pk(e[0], o[0]) for e, o in V], [pk(e[1], o[1]) for e, o in V]


def st_GE(tabs, UE, Gs, Sr, Si, hx):
    tv = [rows(R, hx * (16 * VP), 16 * VP) for R in tabs[1:3]] + [rows(R, hx * 16, 16, 16) for R in tabs[3:9]]
    Gv = rows(Gs, hx * 1024, 1024, 1024)
    Uv = rows(UE, hx * (8 * UP), 8 * UP)
    Srv, Siv = rows(Sr, hx * (8 * SPB), 8 * SPB, 16), rows(Si, hx * (8 * SPB), 8 * SPB, 16)
    for p in range(8):
        r1, i1 = ggen(tv, 2 * p)
        r2, i2 = ggen(tv, 2 * p + 1)
        Gr = jnp.concatenate(r1 + r2, axis=0)
        Gi = jnp.concatenate(i1 + i2, axis=0)
        Gv[pl.ds(p * 128, 64), :] = Gr
        Gv[pl.ds(p * 128 + 64, 64), :] = Gi
        L = bc16(Uv[pl.ds(p * UP, 32), :])
        Srv[pl.ds(p * SPB, 64), :] = jnp.dot(L, bc16(Gr), preferred_element_type=F32).astype(BF16)
        Siv[pl.ds(p * SPB, 64), :] = jnp.dot(L, bc16(Gi), preferred_element_type=F32).astype(BF16)


def st_scan(tabs, Sr, Si, Hr, Hn, hx):
    dtb, V0r, V0i, P1r, P1i, P16r, P16i, P32r, P32i, Lr, Li, Qr, Qi, Wr = tabs
    Hr, Hn = rows(Hr, hx * (8 * HP), 8 * HP), rows(Hn, hx * (8 * HP), 8 * HP)
    W = SPB // 2
    Sv = [R.bitcast(I32).at[pl.ds(pl.multiple_of(hx * (8 * W), 4), 8 * W)] for R in (Sr, Si)]
    lam, first = [], []
    Lr, Li, Qr, Qi = [rows(R, hx * 16, 16, 16) for R in (Lr, Li, Qr, Qi)]
    for ch in range(2):
        sl = pl.ds(ch, 8, stride=2)
        lam.append((Lr[sl, :], Li[sl, :]))
        first.append((Qr[sl, :], -Qi[sl, :]))
    wst = lambda s_: pl.ds(s_, 8, stride=HP)

    def step(ch, sr, si, st):
        if st is None:
            return sr, -si
        H, N = st
        lr, li = lam[ch]
        return (lr * H + sr) + li * N, (lr * N - si) - li * H

    e0, o0 = first
    st0 = st1 = None
    for j in range(16):
        wa = [V[pl.ds(2 * j, 8, stride=W), :] for V in Sv]
        wb = [V[pl.ds(2 * j + 1, 8, stride=W), :] for V in Sv]
        st0 = step(0, lo16(wa[0]), lo16(wa[1]), st0)
        st1 = step(1, hi16(wb[0]), hi16(wb[1]), st1)
        e1, o1 = st0, st1
        Hr[wst(2 * j), :] = pk(e0[0], o1[0])
        Hn[wst(2 * j), :] = pk(e0[1], o1[1])
        Hr[wst(2 * j + 1), :] = pk(e1[0], o0[0])
        Hn[wst(2 * j + 1), :] = pk(e1[1], o0[1])
        if j < 15:
            st0 = step(0, lo16(wb[0]), lo16(wb[1]), st0)
            st1 = step(1, hi16(wa[0]), hi16(wa[1]), st1)
            e0, o0 = st0, st1
        yield


def st_F(Gs, Hr, Hn, Y1s, hx):
    Hr, Hn = rows(Hr, hx * (8 * HP), 8 * HP), rows(Hn, hx * (8 * HP), 8 * HP)
    Gv = rows(Gs, hx * 1024, 1024, 1024)
    for p in range(8):
        hr = bc16(Hr[pl.ds(p * HP, 32), :])
        hn = bc16(Hn[pl.ds(p * HP, 32), :])
        Gr = bc16(Gv[pl.ds(p * 128, 64), :])
        Gi = bc16(Gv[pl.ds(p * 128 + 64, 64), :])
        Y1s[p] = (lax.dot_general(hr, Gr, NT, preferred_element_type=F32)
                  + lax.dot_general(hn, Gi, NT, preferred_element_type=F32))
        yield


def st_T(UE, Y1s, YT, hx):
    l8 = lax.broadcasted_iota(I32, (8, 128), 1)
    r8 = lax.broadcasted_iota(I32, (8, 128), 0)
    rev = 7 - r8
    Uv = rows(UE, hx * (8 * UP), 8 * UP)
    Yv = rows(YT, hx * (8 * YP), 8 * YP, 16)
    for pl_ in range(8):
        top = Y1s[pl_, 0:8, :]
        K1 = jnp.where(l8 < 64, jnp.broadcast_to(top[0:1], (8, 128)), 0.0)
        K2 = jnp.where(l8 >= 64, jnp.broadcast_to(top[3:4], (8, 128)), 0.0)
        tiles = []
        for K in (K1, K2):
            Kp = pk(pltpu.roll(K, 1, 1), K)
            for i in range(4):
                R = pltpu.roll(Kp, 49 - 16 * i, 1, stride=2, stride_axis=0)
                tiles.append(jnp.take_along_axis(R, rev, axis=0, mode="promise_in_bounds"))
        TK = bc16(jnp.concatenate(tiles, axis=0))
        L = bc16(Uv[pl.ds(pl_ * UP, 32), :])
        Y2 = jnp.dot(L, TK, preferred_element_type=F32)
        top = jnp.where((r8 == 0) | (r8 == 3), 0.0, top)
        Y = jnp.concatenate([top, Y1s[pl_, 8:64, :]], axis=0) + Y2
        Yv[pl.ds(pl_ * YP, 64), :] = Y.astype(BF16)
        yield


def ypost(YT, u_s, Dv, b_s, g, jj, e):
    l, m = lane_consts()
    W = YP // 2
    Yv = YT.bitcast(I32).at[pl.ds(pl.multiple_of(g * (64 * W) + 4 * jj, 4), 64 * W - 28)]
    A = jnp.concatenate([Yv[pl.ds(8 * k * W + 2 * e, 8, stride=W), :] for k in range(8)], axis=0)
    B = jnp.concatenate([Yv[pl.ds(8 * k * W + 2 * e + 1, 8, stride=W), :] for k in range(8)], axis=0)
    m64 = jnp.concatenate([m] * 8, axis=0)
    T = (A & m64) | (pltpu.roll(B, 64, 1) & (~m64))
    y = bc16(T).T
    j = 2 * jj + e
    u = ldb(u_s, g, j * 128, 128).astype(F32)
    b_s[g, pl.ds(pl.multiple_of(j * 128, 128), 128), :] = (
        y.astype(F32) + u * Dv[pl.ds(g, 1), :]).astype(BF16)


def wt_prep(w_s, wt_s):
    for c in range(4):
        for i, n in enumerate((0, 1, 2, 3, 8, 9, 10, 11)):
            wt_s.bitcast(I32)[c, 64 * i:64 * i + 64, :] = bc32(ldb(w_s, n, 128 * c, 128).T)
            yield


def kproj_block(x_s, w_s, k_s, b):
    Wk = jnp.concatenate([ldb(w_s, 4 + g, 0, 512) for g in range(4)], axis=1)
    for r in range(512 // KC):
        t0 = b * 512 + KC * r
        X = jnp.concatenate([ldb(x_s, c, t0, KC) for c in range(4)], axis=1)
        Kf = jnp.dot(X, Wk, preferred_element_type=F32)
        for g in range(4):
            k_s[g, pl.ds(pl.multiple_of(t0, KC), KC), :] = Kf[:, 128 * g:128 * g + 128].astype(BF16)
        yield


def qv_step(x_s, wt_s, qT_s, vT_s, j, QC):
    X = jnp.concatenate([ldb(x_s, c, j * TB, TB) for c in range(4)], axis=1)
    for r in range(1024 // QC):
        WT = jnp.concatenate([ldb(wt_s, c, QC * r, QC) for c in range(4)], axis=1)
        QV = lax.dot_general(WT, X, NT, preferred_element_type=F32)
        for b in range(TB // 128):
            i = j * (TB // 128) + b
            blk = QV[:, 128 * b:128 * b + 128]
            if QC * r < 512:
                qT_s[i, QC * r:QC * r + QC, :] = (blk * QSCALE).astype(BF16)
            else:
                vT_s[i, QC * r - 512:QC * r - 512 + QC, :] = blk.astype(BF16)
        yield


def qv_step2(x_s, wt_s, qT_s, vT_s, j):
    for b in range(TB // 128):
        i = j * (TB // 128) + b
        X = jnp.concatenate([ldb(x_s, c, i * 128, 128) for c in range(4)], axis=1)
        for r in range(8):
            WT = jnp.concatenate([ldb(wt_s, c, 128 * r, 128) for c in range(4)], axis=1)
            blk = lax.dot_general(WT, X, NT, preferred_element_type=F32)
            if r < 4:
                qT_s[i, 128 * r:128 * r + 128, :] = (blk * QSCALE).astype(BF16)
            else:
                vT_s[i, 128 * r - 512:128 * r - 384, :] = blk.astype(BF16)
            yield


def interleave(main, side, n_main, n_side, skip=0):
    done = 0
    for i in range(n_main):
        upto = 0 if i < skip else (n_side * (i + 1 - skip)) // (n_main - skip)
        while done < upto:
            next(side, None)
            done += 1
        next(main, None)
    for _ in side:
        pass
    for _ in main:
        pass


def each(fn, items):
    for it in items:
        fn(it)
        yield


def chain(gens, width=1):
    for i in range(0, len(gens), width):
        grp = gens[i:i + width]
        for _ in zip(*grp):
            yield


def wq_tile(qT_s, i, g, h):
    qh = ldb(qT_s, i, (g * 8 + h) * 16, 16)
    parts = []
    if h > 0:
        parts.append(jnp.zeros((16 * h, 128), BF16))
    parts.append(qh)
    if h < 7:
        parts.append(jnp.zeros((16 * (7 - h), 128), BF16))
    return jnp.concatenate(parts, axis=0)


def stage_A(i, g, h0, kind, k_s, qT_s, sw, sy, sm, slot):
    r0 = i * 128
    Wq = jnp.concatenate([wq_tile(qT_s, i, g, h0 + a) for a in range(4)], axis=1)
    parts = []
    if kind == 2:
        for t in range(8):
            parts.append(ldb(k_s, g, r0 - 256 + 16 * t, 16))
            parts.append(ldb(k_s, g, r0 + 16 * t, 16))
        parts.append(ldb(k_s, g, r0 - 128, 128))
    else:
        parts.append(ldb(k_s, g, r0, 128))
        if kind == 1:
            parts.append(ldb(k_s, g, r0 - 128, 128))
    S = jnp.dot(jnp.concatenate(parts, axis=0), Wq, preferred_element_type=F32)
    rows = lax.broadcasted_iota(I32, (16, 128), 0)
    lanes = lax.broadcasted_iota(I32, (16, 128), 1)
    for a in range(4):
        Sa = S[:, a * 128:(a + 1) * 128]
        m = None
        for t in range(8):
            if kind == 2:
                X = Sa[32 * t:32 * t + 16]
                Z = Sa[32 * t + 16:32 * t + 32]
            else:
                X = jnp.full((16, 128), NEG, F32)
                Z = Sa[16 * t:16 * t + 16]
            W = jnp.where(rows + 16 * t <= lanes, Z, X)
            sw[slot, a, 16 * t:16 * t + 16, :] = W
            mm = jnp.maximum(W[:8], W[8:])
            m = mm if m is None else jnp.maximum(m, mm)
        if kind >= 1:
            Y = Sa[256:] if kind == 2 else Sa[128:]
            sy[slot, a] = Y
            for t in range(16):
                m = jnp.maximum(m, Y[8 * t:8 * t + 8])
        sm[slot, a] = m


def stage_A2(i, g, h0, k_s, qT_s, sw, sy, sm, slot):
    l8 = lax.broadcasted_iota(I32, (8, 128), 1)
    lo8 = l8 < 64
    Q = qT_s.bitcast(I32)

    def wtile(h, swap):
        q1 = Q[i, pl.ds((g * 8 + h) * 8, 8), :]
        q2 = Q[i, pl.ds((g * 8 + h + 1) * 8, 8), :]
        z = jnp.zeros_like(q1)
        if swap:
            w1, w2 = jnp.where(lo8, z, q1), jnp.where(lo8, q2, z)
        else:
            w1, w2 = jnp.where(lo8, q1, z), jnp.where(lo8, z, q2)
        parts = []
        if h > 0:
            parts.append(jnp.zeros((16 * h, 128), BF16))
        parts += [bc16(w1), bc16(w2)]
        if h < 6:
            parts.append(jnp.zeros((16 * (6 - h), 128), BF16))
        return jnp.concatenate(parts, axis=0)

    WA = jnp.concatenate([wtile(h0, False), wtile(h0 + 2, False)], axis=1)
    WB = jnp.concatenate([wtile(h0, True), wtile(h0 + 2, True)], axis=1)
    base = pl.multiple_of(i * 64 - 128, 64) if not isinstance(i, int) else i * 64 - 128
    order = (0, 4, 3, 1, 2)
    K = k_s.bitcast(I32).at[g, pl.ds(base, 192), :]
    odd = (l8 & 16) != 0
    LA, LB = [], []
    for t in range(4):
        kk = [K[pl.ds(32 * m + 8 * t, 8), :] for m in range(6)]
        for m in order:
            LA.append(bc16(jnp.where(odd, kk[m + 1], kk[m])))
            LB.append(bc16(jnp.where(odd, kk[m], kk[m + 1])))
    LA = jnp.concatenate(LA, axis=0)
    LB = jnp.concatenate(LB, axis=0)
    SA = jnp.dot(LA, WA, preferred_element_type=F32)
    SB = jnp.dot(LB, WB, preferred_element_type=F32)
    rows = lax.broadcasted_iota(I32, (16, 128), 0)
    lanes = lax.broadcasted_iota(I32, (16, 128), 1)
    lo = lanes < 64
    for pp in range(2):
        m1 = m2 = None
        mx = lambda m, v: jnp.maximum(v[:8], v[8:]) if m is None else jnp.maximum(m, jnp.maximum(v[:8], v[8:]))
        for t in range(4):
            blk = lambda S, m: S[80 * t + 16 * order.index(m):80 * t + 16 * order.index(m) + 16,
                                 128 * pp:128 * pp + 128]
            A = [blk(SA, m) for m in range(5)]
            B = [blk(SB, m) for m in range(5)]
            mk = (lanes & 63) < rows + 16 * t
            MA = jnp.where(mk, A[0], A[4])
            MB = jnp.where(mk, B[0], B[4])
            outs1 = ((sw, 16 * t, jnp.where(lo, MA, B[3])), (sw, 64 + 16 * t, jnp.where(lo, A[1], MB)),
                     (sy, 16 * t, jnp.where(lo, A[2], B[1])), (sy, 64 + 16 * t, jnp.where(lo, A[3], B[2])))
            outs2 = ((sw, 16 * t, jnp.where(lo, MB, A[3])), (sw, 64 + 16 * t, jnp.where(lo, B[1], MA)),
                     (sy, 16 * t, jnp.where(lo, B[2], A[1])), (sy, 64 + 16 * t, jnp.where(lo, B[3], A[2])))
            for ref, r, v in outs1:
                ref[slot, 2 * pp, r:r + 16, :] = v
                m1 = mx(m1, v)
            for ref, r, v in outs2:
                ref[slot, 2 * pp + 1, r:r + 16, :] = v
                m2 = mx(m2, v)
        sm[slot, 2 * pp] = m1
        sm[slot, 2 * pp + 1] = m2


def stage_B(i, g, h0, kind, vT_s, oT_s, sw, sy, sm, slot, oslot):
    lanes = lax.broadcasted_iota(I32, (128, 128), 1)
    rows = lax.broadcasted_iota(I32, (128, 128), 0)
    tri = rows <= lanes
    for a in range(4):
        hh = g * 8 + h0 + a
        m = jnp.max(sm[slot, a], axis=0, keepdims=True)
        pW = jnp.exp2(sw[slot, a] - m)
        vt = lambda blk: ldb(vT_s, blk, hh * 16, 16)
        if kind == 0:
            l = jnp.sum(pW, axis=0, keepdims=True)
            P = pW.astype(BF16)
            Vt = vt(i)
        else:
            pY = jnp.exp2(sy[slot, a] - m)
            l = jnp.sum(pW + pY, axis=0, keepdims=True)
            if kind == 1:
                P = jnp.concatenate([pY, pW], axis=0).astype(BF16)
                Vt = jnp.concatenate([vt(i - 1), vt(i)], axis=1)
            else:
                z = jnp.zeros_like(pW)
                P = jnp.concatenate([jnp.where(tri, z, pW), pY, jnp.where(tri, pW, z)],
                                    axis=0).astype(BF16)
                Vt = jnp.concatenate([vt(i - 2), vt(i - 1), vt(i)], axis=1)
        O = jnp.dot(Vt, P, preferred_element_type=F32) * (1.0 / l)
        oT_s[oslot, hh * 16:(hh + 1) * 16, :] = O.astype(BF16)


def wot_prep(wo_s, wot_s, n):
    for c in range(4):
        wot_s.bitcast(I32)[c, pl.ds(pl.multiple_of(64 * n, 64), 64), :] = bc32(ldb(wo_s, n, 128 * c, 128).T)


def outproj(oT_s, oslot, wot_s, a_s, i):
    WoT = jnp.concatenate([ldb(wot_s, c, 0, 512) for c in range(4)], axis=1)
    AT = jnp.dot(WoT, ldb(oT_s, oslot, 0, 512), preferred_element_type=F32)
    r = pl.ds(pl.multiple_of(i * 64, 64), 64)
    for n in range(4):
        a_s.bitcast(I32)[n, r, :] = bc32(AT[128 * n:128 * n + 128, :].astype(BF16).T)


def kernel_body(x_h, w_h, wo_h, u_h, Are_h, Aim_h, Bre_h, Bim_h, Cre_h, Cim_h, ldt_h, D_h,
                out_h,
                x_s, w_s, wo_s, u_s, Are, Aim, Bre, Bim, Cre, Cim, ldt_v, D_v,
                a_s, b_s, sems,
                wt_s, wot_s, k_s, qT_s, vT_s, oT_s, sw, sy, sm, Dv, *scr):
    tabs = scr[:14]
    UE, Gs, Sr, Si, Hr, Hn, Y1e, Y1o, YT = scr[14:]
    z = pl.program_id(0)

    def copy(src, dst, k):
        return pltpu.make_async_copy(src, dst, sems.at[k])

    def cp_par(r0, n, k):
        return [copy(s.at[pl.ds(r0, n)], d.at[pl.ds(r0, n)], k) for s, d in (
            (Are_h, Are), (Aim_h, Aim), (Bre_h, Bre), (Bim_h, Bim), (Cre_h, Cre), (Cim_h, Cim))]

    cp_w = lambda ns, k: [copy(w_h.at[:, pl.ds(128 * n, 128)], w_s.at[n], k) for n in ns]
    cp_x = lambda r0, n, k: [copy(x_h.at[0, pl.ds(r0, n), pl.ds(128 * c, 128)], x_s.at[c, pl.ds(r0, n), :], k)
                             for c in range(4)]
    cp_wk = cp_w((4, 5, 6, 7), 0)
    cp_x0a, cp_x0b = cp_x(0, 128, 1), cp_x(128, 384, 2)
    cp_x1, cp_x2, cp_x3 = cp_x(512, 512, 3), cp_x(1024, 512, 4), cp_x(1536, 512, 5)
    cp_para = [copy(ldt_h, ldt_v, 6), copy(D_h, D_v, 6)] + cp_par(0, 128, 6)
    cp_parb = cp_par(128, 384, 7)
    cp_wqv = cp_w((0, 1, 2, 3, 8, 9, 10, 11), 10)
    cp_u = [copy(u_h.at[0, :, pl.ds(128 * g, 128)], u_s.at[g], 11) for g in range(4)]
    cp_wo = [copy(wo_h.at[:, pl.ds(128 * n, 128)], wo_s.at[n], 12) for n in range(4)]
    for c in cp_wk + cp_x0a + cp_x0b + cp_x1 + cp_para + cp_x2 + cp_parb + cp_x3 + cp_wqv + cp_u + cp_wo:
        c.start()

    def a_copies(i0, nb):
        r = pl.ds(pl.multiple_of(i0 * 128, 128), 128 * nb)
        return [pltpu.make_async_copy(a_s.at[n, r, :], out_h.at[0, r, pl.ds(128 * n, 128)], sems.at[8])
                for n in range(4)]

    def b_copy(g):
        return pltpu.make_async_copy(b_s.at[g], out_h.at[0, :, pl.ds(DM + 128 * g, 128)], sems.at[9])

    wait = lambda cps: [c.wait() for c in cps]
    params = (Are, Aim, Bre, Bim, Cre, Cim)
    prep = lambda h: prep_hex(params, tabs, h)
    kproj = lambda b: kproj_block(x_s, w_s, k_s, b)
    qv = lambda j, qc: qv_step(x_s, wt_s, qT_s, vT_s, j, qc)
    qv2 = lambda j: qv_step2(x_s, wt_s, qT_s, vT_s, j)
    nk = 512 // KC


    def block(fn):
        @pl.loop(0, 2)
        def _(it):
            @pl.when(it == 1)
            def _():
                fn(it - 1)

    wait(cp_wk + cp_x0a)
    k0 = kproj(0)
    for _ in range(128 // KC):
        next(k0)
    wait(cp_x0b)
    for _ in k0:
        pass
    wait(cp_x1 + cp_para)
    prep_dt(ldt_v, tabs[0])

    @block
    def _(z):
        interleave(kproj(z + 1), each(prep, [z + i for i in range(8)]), nk, 8)

    wait(cp_x2 + cp_parb)

    @block
    def _(z):
        interleave(kproj(z + 2), each(prep, [z + 8 + i for i in range(8)]), nk, 8)

    wait(cp_x3 + cp_wqv)

    def side3(z):
        wt = wt_prep(w_s, wt_s)
        for i in range(NP[0], NP[1]):
            prep(z + i)
            for _ in range(-(-32 // (NP[1] - NP[0]))):
                next(wt, None)
            yield

    @block
    def _(z):
        interleave(kproj(z + 3), side3(z), nk, NP[1] - NP[0])


    @block
    def _(z):
        interleave(qv(z, 128), each(prep, [z + i for i in range(NP[1], NP[2])]), 8, NP[2] - NP[1])

    wait(cp_u)

    def side_b():
        todo = list(range(NP[2], 32))
        for t in range(64):
            if todo and t % 4 == 0:
                prep(z + todo.pop(0))
            uprep(u_s, UE, z + t // 16, z + t % 16)
            yield

    interleave(chain([qv(z + j, 128) for j in (1, 2, 3)]), side_b(), 24, 64)

    def dskip():
        Wr = tabs[13]
        Dv[0:4, :] = D_v[...].astype(F32).reshape(4, 128) + jnp.concatenate(
            [jnp.sum(Wr[128 * g:128 * g + 128, :].T, axis=0, keepdims=True) for g in range(4)], axis=0)

    @pl.loop(0, 32 // UNR_GE)
    def _(q):
        for i in range(UNR_GE):
            st_GE(tabs, UE, Gs, Sr, Si, UNR_GE * q + i)

    wait(cp_wo)

    @pl.loop(0, 4 // UNR_Q2)
    def _(jj):
        for e in range(UNR_Q2):
            j = UNR_Q2 * jj + e
            wot_prep(wo_s, wot_s, j)
            if e == 0:
                dskip()
            interleave(qv2(j + 4),
                       chain([st_scan(tabs, Sr, Si, Hr, Hn, j * 8 + i) for i in range(8)]),
                       16, 16 * 8)

    Y1 = (Y1e, Y1o)
    F = lambda h, par: st_F(Gs, Hr, Hn, Y1[par], h)
    T = lambda h, par: st_T(UE, Y1[par], YT, h)
    run = lambda gens: [None for _ in chain(gens)]
    run([F(z, 0)])

    @pl.loop(0, 32 // UNR_FT - 1)
    def _(q):
        m = UNR_FT * q
        run([g_ for i in range(UNR_FT) for g_ in (F(m + i + 1, (i + 1) % 2), T(m + i, i % 2))])

    m = z + 32 - UNR_FT
    run([g_ for i in range(UNR_FT - 1) for g_ in (F(m + i + 1, (i + 1) % 2), T(m + i, i % 2))]
        + [T(z + 31, 1)])

    steps = [(g, h0) for g in range(4) for h0 in (0, 4)]

    def A(i, s, kind, slot):
        if kind == 2:
            stage_A2(i, *steps[s], k_s, qT_s, sw, sy, sm, slot)
        else:
            stage_A(i, *steps[s], kind, k_s, qT_s, sw, sy, sm, slot)

    B = lambda i, s, kind, slot, osl: stage_B(i, *steps[s], kind, vT_s, oT_s, sw, sy, sm, slot, osl)

    def yp(t0, c):
        t = t0 + c
        ypost(YT, u_s, Dv, b_s, t >> 4, (t & 15) >> 1, c % 2)

    A(0, 0, 0, 0)
    for s in range(8):
        if s % 4 == 0:
            yp(z, s // 4)
        if s < 7:
            A(0, s + 1, 0, (s + 1) % 2)
        else:
            A(1, 0, 1, 0)
        B(0, s, 0, s % 2, 0)
    for s in range(8):
        if s % 4 == 0:
            yp(z + 2, s // 4)
        if s < 7:
            A(1, s + 1, 1, (s + 1) % 2)
        else:
            A(2, 0, 2, 0)
        B(1, s, 1, s % 2, 1)
        if s == 1:
            outproj(oT_s, 0, wot_s, a_s, 0)

    def att_pair(i0, t0, last):
        for e in range(2):
            i = i0 + e
            for s in range(8):
                if t0 is not None and s < 5:
                    yp(t0, 5 * e + s)
                if s < 7:
                    A(i, s + 1, 2, (s + 1) % 2)
                elif not (last and e == 1):
                    A(i + 1, 0, 2, 0)
                B(i, s, 2, s % 2, e)
                if s == 1:
                    outproj(oT_s, 1 - e, wot_s, a_s, i - 1)

    start = lambda cps: [c.start() for c in cps]

    start(a_copies(0, 1))

    @pl.loop(0, 3)
    def _(it):
        i0 = 2 + 4 * it
        att_pair(i0, 4 + 20 * it, False)
        att_pair(i0 + 2, 14 + 20 * it, False)
        start(a_copies(i0 - 1, 4) + [b_copy(it)])

        @pl.when(it == 2)
        def _():
            b_copy(3).start()

    @block
    def _(z):
        att_pair(z + 14, None, True)
        start(a_copies(13, 2))

    outproj(oT_s, 1, wot_s, a_s, z + 15)
    start(a_copies(15, 1))
    for g in range(4):
        b_copy(g).wait()
    wait(a_copies(0, 1) + a_copies(1, 4) + a_copies(5, 4) + a_copies(9, 4) + a_copies(13, 2) + a_copies(15, 1))


def _scratch():
    T = lambda r: pltpu.VMEM((r, 128), F32)
    V = pltpu.VMEM
    s = [V((4, SEQ, 128), BF16), V((12, DM, 128), BF16), V((4, DM, 128), BF16), V((4, SEQ, 128), BF16)]
    s += [V((DM, 128), BF16)] * 6 + [V((DM,), BF16)] * 2
    s += [V((4, SEQ, 128), BF16), V((4, SEQ, 128), BF16), pltpu.SemaphoreType.DMA((13,))]
    s += [V((4, 1024, 128), BF16), V((4, DM, 128), BF16), V((4, SEQ, 128), BF16), V((16, DM, 128), BF16), V((16, DM, 128), BF16),
          V((2, DM, 128), BF16), V((2, 4, 128, 128), F32), V((2, 4, 128, 128), F32), V((2, 4, 8, 128), F32),
          T(8)]
    s += [T(512), T(512 * VP), T(512 * VP)] + [T(512)] * 11
    s += [V((256 * UP, 128), I32), V((256 * 128, 128), I32),
          V((256 * SPB, 128), BF16), V((256 * SPB, 128), BF16),
          V((256 * HP, 128), I32), V((256 * HP, 128), I32),
          V((8, 64, 128), F32), V((8, 64, 128), F32), V((256 * YP, 128), BF16)]
    return s


@jax.jit
def pallas_concat_heads__sliding_block__ssm_conv_s4__prompt_kernel(
    A_x: jax.Array,
    A_wqkv: jax.Array,
    A_wo: jax.Array,
    B_u: jax.Array,
    B_A_re: jax.Array,
    B_A_im: jax.Array,
    B_B_re: jax.Array,
    B_B_im: jax.Array,
    B_C_re: jax.Array,
    B_C_im: jax.Array,
    B_log_dt: jax.Array,
    B_Dskip: jax.Array,
):
    hbm = pl.BlockSpec(memory_space=pl.ANY)
    return pl.pallas_call(
        kernel_body,
        grid=(1,),
        in_specs=[hbm] * 12,
        out_specs=hbm,
        out_shape=jax.ShapeDtypeStruct((1, SEQ, 2 * DM), BF16),
        scratch_shapes=_scratch(),
        compiler_params=pltpu.CompilerParams(vmem_limit_bytes=110 * 1024 * 1024),
    )(A_x, A_wqkv, A_wo, B_u, B_A_re, B_A_im, B_B_re, B_B_im, B_C_re, B_C_im, B_log_dt, B_Dskip)
```

```python
import math

import jax
import jax.numpy as jnp
from jax import lax
import jax.experimental.pallas as pl
import jax.experimental.pallas.tpu as pltpu

F32 = jnp.float32
BF16 = jnp.bfloat16
I32 = jnp.int32
NT = (((1,), (1,)), ((), ()))

SEQ = 2048
DM = 512
QSCALE = 0.25 * math.log2(math.e)
NEG = -1e30

UP = 33
HP = 33
SPB = 72
YP = 72
VP = 9
TB = 256
UNR_FT = 16
NP = (16, 24, 32)
UNR_Q2 = 2
KC = 64
UNR_GE = 16


def bc16(x):
    return pltpu.bitcast(x, BF16)


def bc32(x):
    return pltpu.bitcast(x, I32)


def pk(lo, hi):
    return pltpu.pack_elementwise([lo, hi], packed_dtype=BF16)


def lo16(w):
    return pltpu.bitcast(w << 16, F32)


def hi16(w):
    return pltpu.bitcast(w & (-0x10000), F32)


def cmul(ar, ai, br, bi):
    return ar * br - ai * bi, ar * bi + ai * br


def ldb(ref, *idx):
    *lead, r0, n = idx
    if isinstance(r0, int):
        s = pl.ds(r0 // 2, n // 2)
    else:
        s = pl.ds(pl.multiple_of(r0 >> 1, 8), n // 2)
    return bc16(ref.bitcast(I32)[(*lead, s, slice(None))])


def rows(ref, start, n, mult=None):
    if mult is not None:
        start = pl.multiple_of(start, mult)
    return ref.at[pl.ds(start, n)]


def prep_dt(logdt_ref, dtb):
    ld = logdt_ref[...].astype(F32).reshape(4, 128)
    dt = jnp.exp(ld).astype(BF16).astype(F32)
    for g in range(4):
        dtb[128 * g:128 * g + 128, :] = jnp.broadcast_to(dt[g:g + 1, :], (128, 128)).T


def csqrt(a, b):
    aa = jnp.abs(a)
    ab = jnp.abs(b)
    m = jnp.maximum(aa, ab)
    z = m == 0.0
    ms = jnp.where(z, 1.0, m)
    inv = 1.0 / ms
    an = aa * inv
    bn = ab * inv
    r = jnp.sqrt(an * an + bn * bn)
    tn = jnp.sqrt((r + an) * 0.5)
    tn = jnp.where(z, 1.0, tn)
    sm = jnp.sqrt(ms)
    t = tn * sm
    o = (bn / (2.0 * tn)) * sm
    sgn = jnp.where(b < 0, -1.0, 1.0)
    pos = a >= 0
    sr = jnp.where(pos, t, o)
    si = jnp.where(pos, o, t) * sgn
    return jnp.where(z, 0.0, sr), jnp.where(z, 0.0, si)


def prep_hex(params, tabs, h):
    Are, Aim, Bre, Bim, Cre, Cim = params
    dtb, V0r, V0i, P1r, P1i, P16r, P16i, P32r, P32i, Lr, Li, Qr, Qi, Wr = tabs
    rs = pl.ds(pl.multiple_of(h * 16, 16), 16)
    ld = lambda R: ldb(R, h * 16, 16).astype(F32)
    d = dtb[rs, :]
    zr = d * ld(Are)
    zi = d * ld(Aim)
    mag = jnp.exp(zr)
    e1r = mag * jnp.cos(zi)
    e1i = mag * jnp.sin(zi)
    wr, wi = cmul(ld(Cre), ld(Cim), d * ld(Bre), d * ld(Bim))
    w1r, w1i = cmul(wr, wi, e1r, e1i)
    sr, si = csqrt(w1r, w1i)
    Wr[rs, :] = wr
    Qr[rs, :] = sr
    Qi[rs, :] = si
    p2 = cmul(e1r, e1i, e1r, e1i)
    p4 = cmul(*p2, *p2)
    p8 = cmul(*p4, *p4)
    p16 = cmul(*p8, *p8)
    p32 = cmul(*p16, *p16)
    p64 = cmul(*p32, *p32)
    q0 = (sr, si)
    q1 = cmul(*q0, *p2)
    q2 = cmul(*q0, *p4)
    q3 = cmul(*q1, *p4)
    Q = [q0, q1, q2, q3] + [cmul(*q, *p8) for q in (q0, q1, q2, q3)]
    V0rv, V0iv = rows(V0r, h * (16 * VP), 16 * VP), rows(V0i, h * (16 * VP), 16 * VP)
    for j in range(8):
        for half in range(2):
            st = pl.ds(half * 8 * VP + j, 8, stride=VP)
            V0rv[st, :] = Q[j][0][8 * half:8 * half + 8]
            V0iv[st, :] = Q[j][1][8 * half:8 * half + 8]
    P1r[rs, :] = e1r
    P1i[rs, :] = e1i
    P16r[rs, :] = p16[0]
    P16i[rs, :] = p16[1]
    P32r[rs, :] = p32[0]
    P32i[rs, :] = p32[1]
    Lr[rs, :] = p64[0]
    Li[rs, :] = p64[1]


def lane_consts():
    l = lax.broadcasted_iota(I32, (8, 128), 1)
    m = jnp.where(l < 64, 0x0000FFFF, -0x10000).astype(I32)
    return l, m


def uprep(u_s, UE, g, j):
    l, m = lane_consts()
    rev = 7 - lax.broadcasted_iota(I32, (8, 128), 0)
    U = u_s.bitcast(I32).at[g, pl.ds(pl.multiple_of(64 * j, 64), 64), :]
    parts = []
    for c in range(2):
        for v in range(4):
            w = jnp.take_along_axis(U[pl.ds(32 * c + 8 * (3 - v), 8), :], rev, axis=0, mode="promise_in_bounds")
            parts.append((w << 16) | lax.shift_right_logical(w, 16))
    T = bc32(bc16(jnp.concatenate(parts, axis=0)).T)
    UEv = rows(UE, 64 * UP * g + 2 * j, 63 * UP + 2)
    for k in range(8):
        v = T[8 * k:8 * k + 8]
        UEv[pl.ds(8 * k * UP, 8, stride=UP), :] = v & m
        UEv[pl.ds(8 * k * UP + 1, 8, stride=UP), :] = pltpu.roll(v, 64, 1) & m


def ggen(tv, c):
    V0r, V0i, P1r, P1i, P16r, P16i, P32r, P32i = tv
    ve = (V0r[pl.ds(c * VP, 8), :], V0i[pl.ds(c * VP, 8), :])
    row = lambda R: R[pl.ds(c, 1), :]
    p1 = (row(P1r), row(P1i))
    p16 = (row(P16r), row(P16i))
    p32 = (row(P32r), row(P32i))
    vo = cmul(*ve, *p1)
    V = [(ve, vo), (cmul(*ve, *p16), cmul(*vo, *p16))]
    V = V + [(cmul(*e, *p32), cmul(*o, *p32)) for e, o in V]
    return [pk(e[0], o[0]) for e, o in V], [pk(e[1], o[1]) for e, o in V]


def st_GE(tabs, UE, Gs, Sr, Si, hx):
    tv = [rows(R, hx * (16 * VP), 16 * VP) for R in tabs[1:3]] + [rows(R, hx * 16, 16, 16) for R in tabs[3:9]]
    Gv = rows(Gs, hx * 1024, 1024, 1024)
    Uv = rows(UE, hx * (8 * UP), 8 * UP)
    Srv, Siv = rows(Sr, hx * (8 * SPB), 8 * SPB, 16), rows(Si, hx * (8 * SPB), 8 * SPB, 16)
    for p in range(8):
        r1, i1 = ggen(tv, 2 * p)
        r2, i2 = ggen(tv, 2 * p + 1)
        Gr = jnp.concatenate(r1 + r2, axis=0)
        Gi = jnp.concatenate(i1 + i2, axis=0)
        Gv[pl.ds(p * 128, 64), :] = Gr
        Gv[pl.ds(p * 128 + 64, 64), :] = Gi
        L = bc16(Uv[pl.ds(p * UP, 32), :])
        Srv[pl.ds(p * SPB, 64), :] = jnp.dot(L, bc16(Gr), preferred_element_type=F32).astype(BF16)
        Siv[pl.ds(p * SPB, 64), :] = jnp.dot(L, bc16(Gi), preferred_element_type=F32).astype(BF16)


def st_scan(tabs, Sr, Si, Hr, Hn, hx):
    dtb, V0r, V0i, P1r, P1i, P16r, P16i, P32r, P32i, Lr, Li, Qr, Qi, Wr = tabs
    Hr, Hn = rows(Hr, hx * (8 * HP), 8 * HP), rows(Hn, hx * (8 * HP), 8 * HP)
    W = SPB // 2
    Sv = [R.bitcast(I32).at[pl.ds(pl.multiple_of(hx * (8 * W), 4), 8 * W)] for R in (Sr, Si)]
    lam, first = [], []
    Lr, Li, Qr, Qi = [rows(R, hx * 16, 16, 16) for R in (Lr, Li, Qr, Qi)]
    for ch in range(2):
        sl = pl.ds(ch, 8, stride=2)
        lam.append((Lr[sl, :], Li[sl, :]))
        first.append((Qr[sl, :], -Qi[sl, :]))
    wst = lambda s_: pl.ds(s_, 8, stride=HP)

    def step(ch, sr, si, st):
        if st is None:
            return sr, -si
        H, N = st
        lr, li = lam[ch]
        return (lr * H + sr) + li * N, (lr * N - si) - li * H

    e0, o0 = first
    st0 = st1 = None
    for j in range(16):
        wa = [V[pl.ds(2 * j, 8, stride=W), :] for V in Sv]
        wb = [V[pl.ds(2 * j + 1, 8, stride=W), :] for V in Sv]
        st0 = step(0, lo16(wa[0]), lo16(wa[1]), st0)
        st1 = step(1, hi16(wb[0]), hi16(wb[1]), st1)
        e1, o1 = st0, st1
        Hr[wst(2 * j), :] = pk(e0[0], o1[0])
        Hn[wst(2 * j), :] = pk(e0[1], o1[1])
        Hr[wst(2 * j + 1), :] = pk(e1[0], o0[0])
        Hn[wst(2 * j + 1), :] = pk(e1[1], o0[1])
        if j < 15:
            st0 = step(0, lo16(wb[0]), lo16(wb[1]), st0)
            st1 = step(1, hi16(wa[0]), hi16(wa[1]), st1)
            e0, o0 = st0, st1
        yield


def st_F(Gs, Hr, Hn, Y1s, hx):
    Hr, Hn = rows(Hr, hx * (8 * HP), 8 * HP), rows(Hn, hx * (8 * HP), 8 * HP)
    Gv = rows(Gs, hx * 1024, 1024, 1024)
    for p in range(8):
        hr = bc16(Hr[pl.ds(p * HP, 32), :])
        hn = bc16(Hn[pl.ds(p * HP, 32), :])
        Gr = bc16(Gv[pl.ds(p * 128, 64), :])
        Gi = bc16(Gv[pl.ds(p * 128 + 64, 64), :])
        Y1s[p] = (lax.dot_general(hr, Gr, NT, preferred_element_type=F32)
                  + lax.dot_general(hn, Gi, NT, preferred_element_type=F32))
        yield


def st_T(UE, Y1s, YT, hx):
    l8 = lax.broadcasted_iota(I32, (8, 128), 1)
    r8 = lax.broadcasted_iota(I32, (8, 128), 0)
    rev = 7 - r8
    Uv = rows(UE, hx * (8 * UP), 8 * UP)
    Yv = rows(YT, hx * (8 * YP), 8 * YP, 16)
    for pl_ in range(8):
        top = Y1s[pl_, 0:8, :]
        K1 = jnp.where(l8 < 64, jnp.broadcast_to(top[0:1], (8, 128)), 0.0)
        K2 = jnp.where(l8 >= 64, jnp.broadcast_to(top[3:4], (8, 128)), 0.0)
        tiles = []
        for K in (K1, K2):
            Kp = pk(pltpu.roll(K, 1, 1), K)
            for i in range(4):
                R = pltpu.roll(Kp, 49 - 16 * i, 1, stride=2, stride_axis=0)
                tiles.append(jnp.take_along_axis(R, rev, axis=0, mode="promise_in_bounds"))
        TK = bc16(jnp.concatenate(tiles, axis=0))
        L = bc16(Uv[pl.ds(pl_ * UP, 32), :])
        Y2 = jnp.dot(L, TK, preferred_element_type=F32)
        top = jnp.where((r8 == 0) | (r8 == 3), 0.0, top)
        Y = jnp.concatenate([top, Y1s[pl_, 8:64, :]], axis=0) + Y2
        Yv[pl.ds(pl_ * YP, 64), :] = Y.astype(BF16)
        yield


def ypost(YT, u_s, Dv, b_s, g, jj, e):
    l, m = lane_consts()
    W = YP // 2
    Yv = YT.bitcast(I32).at[pl.ds(pl.multiple_of(g * (64 * W) + 4 * jj, 4), 64 * W - 28)]
    A = jnp.concatenate([Yv[pl.ds(8 * k * W + 2 * e, 8, stride=W), :] for k in range(8)], axis=0)
    B = jnp.concatenate([Yv[pl.ds(8 * k * W + 2 * e + 1, 8, stride=W), :] for k in range(8)], axis=0)
    m64 = jnp.concatenate([m] * 8, axis=0)
    T = (A & m64) | (pltpu.roll(B, 64, 1) & (~m64))
    y = bc16(T).T
    j = 2 * jj + e
    u = ldb(u_s, g, j * 128, 128).astype(F32)
    b_s[g, pl.ds(pl.multiple_of(j * 128, 128), 128), :] = (
        y.astype(F32) + u * Dv[pl.ds(g, 1), :]).astype(BF16)


def wt_prep(w_s, wt_s):
    for c in range(4):
        for i, n in enumerate((0, 1, 2, 3, 8, 9, 10, 11)):
            wt_s.bitcast(I32)[c, 64 * i:64 * i + 64, :] = bc32(ldb(w_s, n, 128 * c, 128).T)
            yield


def kproj_block(x_s, w_s, k_s, b):
    Wk = jnp.concatenate([ldb(w_s, 4 + g, 0, 512) for g in range(4)], axis=1)
    for r in range(512 // KC):
        t0 = b * 512 + KC * r
        X = jnp.concatenate([ldb(x_s, c, t0, KC) for c in range(4)], axis=1)
        Kf = jnp.dot(X, Wk, preferred_element_type=F32)
        for g in range(4):
            k_s[g, pl.ds(pl.multiple_of(t0, KC), KC), :] = Kf[:, 128 * g:128 * g + 128].astype(BF16)
        yield


def xperm(x, s):
    if s == 0:
        return x
    if s == 64:
        return pltpu.roll(x, 64, 1)
    l8 = lax.broadcasted_iota(I32, (8, 128), 1)
    up = ((l8 & 32) != 0) if s == 32 else ((l8 & 32) == 0)
    return jnp.where(up, pltpu.roll(x, 32, 1), pltpu.roll(x, 96, 1))


def store_q(qT_s, i, r0, blk, perm):
    v = (blk * QSCALE).astype(BF16)
    if not perm:
        qT_s[i, r0:r0 + 128, :] = v
        return
    v = bc32(v)
    for h in range(8):
        qT_s.bitcast(I32)[i, pl.ds(r0 // 2 + 8 * h, 8), :] = xperm(v[8 * h:8 * h + 8], 32 * (h % 4) if perm else 0)


def qperm(qT_s, i):
    Q = qT_s.bitcast(I32)
    for h in range(32):
        if h % 4:
            Q[i, 8 * h:8 * h + 8, :] = xperm(Q[i, 8 * h:8 * h + 8, :], 32 * (h % 4))


def qv_step(x_s, wt_s, qT_s, vT_s, j, QC, perm):
    X = jnp.concatenate([ldb(x_s, c, j * TB, TB) for c in range(4)], axis=1)
    for r in range(1024 // QC):
        WT = jnp.concatenate([ldb(wt_s, c, QC * r, QC) for c in range(4)], axis=1)
        QV = lax.dot_general(WT, X, NT, preferred_element_type=F32)
        for b in range(TB // 128):
            i = j * (TB // 128) + b
            blk = QV[:, 128 * b:128 * b + 128]
            if QC * r < 512:
                store_q(qT_s, i, QC * r, blk, perm)
            else:
                vT_s[i, QC * r - 512:QC * r - 512 + QC, :] = blk.astype(BF16)
        yield


def qv_step2(x_s, wt_s, qT_s, vT_s, j):
    for b in range(TB // 128):
        i = j * (TB // 128) + b
        X = jnp.concatenate([ldb(x_s, c, i * 128, 128) for c in range(4)], axis=1)
        for r in range(8):
            WT = jnp.concatenate([ldb(wt_s, c, 128 * r, 128) for c in range(4)], axis=1)
            blk = lax.dot_general(WT, X, NT, preferred_element_type=F32)
            if r < 4:
                store_q(qT_s, i, 128 * r, blk, False)
            else:
                vT_s[i, 128 * r - 512:128 * r - 384, :] = blk.astype(BF16)
            yield


def interleave(main, side, n_main, n_side, skip=0):
    done = 0
    for i in range(n_main):
        upto = 0 if i < skip else (n_side * (i + 1 - skip)) // (n_main - skip)
        while done < upto:
            next(side, None)
            done += 1
        next(main, None)
    for _ in side:
        pass
    for _ in main:
        pass


def each(fn, items):
    for it in items:
        fn(it)
        yield


def chain(gens, width=1):
    for i in range(0, len(gens), width):
        grp = gens[i:i + width]
        for _ in zip(*grp):
            yield


def wq_tile(qT_s, i, g, h):
    qh = ldb(qT_s, i, (g * 8 + h) * 16, 16)
    parts = []
    if h > 0:
        parts.append(jnp.zeros((16 * h, 128), BF16))
    parts.append(qh)
    if h < 7:
        parts.append(jnp.zeros((16 * (7 - h), 128), BF16))
    return jnp.concatenate(parts, axis=0)


def stage_A(i, g, h0, kind, k_s, qT_s, sw, sy, sm, slot):
    r0 = i * 128
    Wq = jnp.concatenate([wq_tile(qT_s, i, g, h0 + a) for a in range(4)], axis=1)
    parts = []
    parts.append(ldb(k_s, g, r0, 128))
    if kind == 1:
        parts.append(ldb(k_s, g, r0 - 128, 128))
    S = jnp.dot(jnp.concatenate(parts, axis=0), Wq, preferred_element_type=F32)
    rows = lax.broadcasted_iota(I32, (16, 128), 0)
    lanes = lax.broadcasted_iota(I32, (16, 128), 1)
    for a in range(4):
        Sa = S[:, a * 128:(a + 1) * 128]
        m = None
        for t in range(8):
            X = jnp.full((16, 128), NEG, F32)
            Z = Sa[16 * t:16 * t + 16]
            W = jnp.where(rows + 16 * t <= lanes, Z, X)
            sw[slot, a, 16 * t:16 * t + 16, :] = W
            mm = jnp.maximum(W[:8], W[8:])
            m = mm if m is None else jnp.maximum(m, mm)
        if kind >= 1:
            Y = Sa[128:]
            sy[slot, a] = Y
            for t in range(16):
                m = jnp.maximum(m, Y[8 * t:8 * t + 8])
        sm[slot, a] = m


def stage_A4(i, g, h0, k_s, qT_s, sw, sy, sm, slot):
    l8 = lax.broadcasted_iota(I32, (8, 128), 1)
    grp = l8 >> 5
    Q = qT_s.bitcast(I32)
    qp = [Q[i, pl.ds((g * 8 + h0 + a) * 8, 8), :] for a in range(4)]
    z = jnp.zeros_like(qp[0])
    pad = jnp.zeros((64, 128), BF16)
    base = pl.multiple_of(i * 64 - 128, 64) if not isinstance(i, int) else i * 64 - 128
    K = k_s.bitcast(I32).at[g, pl.ds(base, 192), :]
    kb = lambda b: bc16(K[pl.ds(16 * b, 16), :])
    S = []
    for j in range(4):
        w = [bc16(jnp.where(grp == (a ^ j), qp[a], z)) for a in range(4)]
        W = jnp.concatenate(w + [pad] if h0 == 0 else [pad] + w, axis=0)
        bands = []
        for c in range(8):
            rho = (c - j) % 8
            bands += (j, j + 8) if rho == 0 else (j + rho,)
        R = jnp.dot(jnp.concatenate([kb(b) for b in bands], axis=0), W, preferred_element_type=F32)
        S.append({b: R[32 * n:32 * n + 32] for n, b in enumerate(bands)})
    rows = lax.broadcasted_iota(I32, (8, 128), 0)
    odd = (l8 & 32) != 0
    top = (l8 & 64) != 0
    m = [None] * 4
    for c in range(8):
        for v in range(4):
            part = lambda j, b: S[j][b][8 * v:8 * v + 8]
            src = []
            for j in range(4):
                rho = (c - j) % 8
                if rho == 0:
                    src.append(jnp.where(rows + 8 * v > (l8 & 31), part(j, j), part(j, j + 8)))
                else:
                    src.append(part(j, j + rho))
            U = [jnp.where(odd, src[j ^ 1], src[j]) for j in range(4)]
            for a in range(4):
                E = jnp.where(top, U[a ^ 2], U[a])
                (sw if c < 4 else sy)[slot, a, pl.ds(32 * (c % 4) + 8 * v, 8), :] = E
                m[a] = E if m[a] is None else jnp.maximum(m[a], E)
    for a in range(4):
        sm[slot, a] = m[a]


def stage_B(i, g, h0, kind, vT_s, oT_s, sw, sy, sm, slot, oslot):
    lanes = lax.broadcasted_iota(I32, (128, 128), 1)
    rows = lax.broadcasted_iota(I32, (128, 128), 0)
    for a in range(4):
        px = 32 * a if kind == 2 else 0
        tri = rows <= (lanes ^ px)
        hh = g * 8 + h0 + a
        m = jnp.max(sm[slot, a], axis=0, keepdims=True)
        pW = jnp.exp2(sw[slot, a] - m)
        vt = lambda blk: ldb(vT_s, blk, hh * 16, 16)
        if kind == 0:
            l = jnp.sum(pW, axis=0, keepdims=True)
            P = pW.astype(BF16)
            Vt = vt(i)
        else:
            pY = jnp.exp2(sy[slot, a] - m)
            l = jnp.sum(pW + pY, axis=0, keepdims=True)
            if kind == 1:
                P = jnp.concatenate([pY, pW], axis=0).astype(BF16)
                Vt = jnp.concatenate([vt(i - 1), vt(i)], axis=1)
            else:
                z = jnp.zeros_like(pW)
                P = jnp.concatenate([pY, jnp.where(tri, z, pW), jnp.where(tri, pW, z)],
                                    axis=0).astype(BF16)
                Vt = jnp.concatenate([vt(i - 1), vt(i - 2), vt(i)], axis=1)
        O = jnp.dot(Vt, P, preferred_element_type=F32) * (1.0 / l)
        oT_s.bitcast(I32)[oslot, hh * 8:(hh + 1) * 8, :] = xperm(bc32(O.astype(BF16)), px)


def wot_prep(wo_s, wot_s, n):
    for c in range(4):
        wot_s.bitcast(I32)[c, pl.ds(pl.multiple_of(64 * n, 64), 64), :] = bc32(ldb(wo_s, n, 128 * c, 128).T)


def outproj(oT_s, oslot, wot_s, a_s, i):
    WoT = jnp.concatenate([ldb(wot_s, c, 0, 512) for c in range(4)], axis=1)
    AT = jnp.dot(WoT, ldb(oT_s, oslot, 0, 512), preferred_element_type=F32)
    r = pl.ds(pl.multiple_of(i * 64, 64), 64)
    for n in range(4):
        a_s.bitcast(I32)[n, r, :] = bc32(AT[128 * n:128 * n + 128, :].astype(BF16).T)


def kernel_body(x_h, w_h, wo_h, u_h, Are_h, Aim_h, Bre_h, Bim_h, Cre_h, Cim_h, ldt_h, D_h,
                out_h,
                x_s, w_s, wo_s, u_s, Are, Aim, Bre, Bim, Cre, Cim, ldt_v, D_v,
                a_s, b_s, sems,
                wt_s, wot_s, k_s, qT_s, vT_s, oT_s, sw, sy, sm, Dv, *scr):
    tabs = scr[:14]
    UE, Gs, Sr, Si, Hr, Hn, Y1e, Y1o, YT = scr[14:]
    z = pl.program_id(0)

    def copy(src, dst, k):
        return pltpu.make_async_copy(src, dst, sems.at[k])

    def cp_par(r0, n, k):
        return [copy(s.at[pl.ds(r0, n)], d.at[pl.ds(r0, n)], k) for s, d in (
            (Are_h, Are), (Aim_h, Aim), (Bre_h, Bre), (Bim_h, Bim), (Cre_h, Cre), (Cim_h, Cim))]

    cp_w = lambda ns, k: [copy(w_h.at[:, pl.ds(128 * n, 128)], w_s.at[n], k) for n in ns]
    cp_x = lambda r0, n, k: [copy(x_h.at[0, pl.ds(r0, n), pl.ds(128 * c, 128)], x_s.at[c, pl.ds(r0, n), :], k)
                             for c in range(4)]
    cp_wk = [copy(ldt_h, ldt_v, 0)] + cp_w((4, 5, 6, 7), 0)
    cp_x0a, cp_x0b = cp_x(0, 128, 1), cp_x(128, 384, 2)
    cp_x1, cp_x2, cp_x3 = cp_x(512, 512, 3), cp_x(1024, 512, 4), cp_x(1536, 512, 5)
    cp_para = [copy(D_h, D_v, 6)] + cp_par(0, 128, 6)
    cp_parb = cp_par(128, 384, 7)
    cp_wqv = cp_w((0, 1, 2, 3, 8, 9, 10, 11), 10)
    cp_u = [copy(u_h.at[0, :, pl.ds(128 * g, 128)], u_s.at[g], 11) for g in range(4)]
    cp_wo = [copy(wo_h.at[:, pl.ds(128 * n, 128)], wo_s.at[n], 12) for n in range(4)]
    for c in cp_wk + cp_x0a + cp_x0b + cp_x1 + cp_para + cp_x2 + cp_parb + cp_x3 + cp_wqv + cp_u + cp_wo:
        c.start()

    def a_copies(i0, nb):
        r = pl.ds(pl.multiple_of(i0 * 128, 128), 128 * nb)
        return [pltpu.make_async_copy(a_s.at[n, r, :], out_h.at[0, r, pl.ds(128 * n, 128)], sems.at[8])
                for n in range(4)]

    def b_copy(g):
        return pltpu.make_async_copy(b_s.at[g], out_h.at[0, :, pl.ds(DM + 128 * g, 128)], sems.at[9])

    wait = lambda cps: [c.wait() for c in cps]
    params = (Are, Aim, Bre, Bim, Cre, Cim)
    prep = lambda h: prep_hex(params, tabs, h)
    kproj = lambda b: kproj_block(x_s, w_s, k_s, b)
    qv = lambda j, qc, perm: qv_step(x_s, wt_s, qT_s, vT_s, j, qc, perm)
    qv2 = lambda j: qv_step2(x_s, wt_s, qT_s, vT_s, j)
    nk = 512 // KC


    def block(fn):
        @pl.loop(0, 2)
        def _(it):
            @pl.when(it == 1)
            def _():
                fn(it - 1)

    wait(cp_wk + cp_x0a)
    prep_dt(ldt_v, tabs[0])
    k0 = kproj(0)
    for _ in range(128 // KC):
        next(k0)
    wait(cp_x0b)
    for _ in k0:
        pass
    wait(cp_x1 + cp_para)

    def side3(z):
        wt = wt_prep(w_s, wt_s)
        for i in range(NP[0], NP[1]):
            prep(z + i)
            for _ in range(-(-32 // (NP[1] - NP[0]))):
                next(wt, None)
            yield

    @block
    def _(z):
        interleave(kproj(z + 1), each(prep, [z + i for i in range(8)]), nk, 8)
        wait(cp_x2 + cp_parb)
        interleave(kproj(z + 2), each(prep, [z + 8 + i for i in range(8)]), nk, 8)

    wait(cp_x3 + cp_wqv)

    @block
    def _(z):
        interleave(kproj(z + 3), side3(z), nk, NP[1] - NP[0])
        interleave(qv(z, 128, False), each(prep, [z + i for i in range(NP[1], NP[2])]), 8, NP[2] - NP[1])

    wait(cp_u)

    def side_b():
        todo = list(range(NP[2], 32))
        for t in range(64):
            if todo and t % 4 == 0:
                prep(z + todo.pop(0))
            uprep(u_s, UE, z + t // 16, z + t % 16)
            yield

    interleave(chain([qv(z + j, 128, True) for j in (1, 2, 3)]), side_b(), 24, 64)

    def dskip():
        Wr = tabs[13]
        Dv[0:4, :] = D_v[...].astype(F32).reshape(4, 128) + jnp.concatenate(
            [jnp.sum(Wr[128 * g:128 * g + 128, :].T, axis=0, keepdims=True) for g in range(4)], axis=0)

    @pl.loop(0, 32 // UNR_GE)
    def _(q):
        for i in range(UNR_GE):
            st_GE(tabs, UE, Gs, Sr, Si, UNR_GE * q + i)

    wait(cp_wo)

    @pl.loop(0, 4 // UNR_Q2)
    def _(jj):
        for e in range(UNR_Q2):
            j = UNR_Q2 * jj + e
            wot_prep(wo_s, wot_s, j)
            if e == 0:
                dskip()
            interleave(qv2(j + 4),
                       chain([st_scan(tabs, Sr, Si, Hr, Hn, j * 8 + i) for i in range(8)]),
                       16, 16 * 8)

    Y1 = (Y1e, Y1o)
    F = lambda h, par: st_F(Gs, Hr, Hn, Y1[par], h)
    T = lambda h, par: st_T(UE, Y1[par], YT, h)
    run = lambda gens: [None for _ in chain(gens)]
    run([F(z, 0)])

    @pl.loop(0, 32 // UNR_FT - 1)
    def _(q):
        m = UNR_FT * q
        for i in range(UNR_FT):
            if i % 2 == 0:
                qperm(qT_s, q + 8 + i // 2)
            run([F(m + i + 1, (i + 1) % 2), T(m + i, i % 2)])

    m = z + 32 - UNR_FT
    run([g_ for i in range(UNR_FT - 1) for g_ in (F(m + i + 1, (i + 1) % 2), T(m + i, i % 2))]
        + [T(z + 31, 1)])

    steps = [(g, h0) for g in range(4) for h0 in (0, 4)]

    def A(i, s, kind, slot):
        if kind == 2:
            stage_A4(i, *steps[s], k_s, qT_s, sw, sy, sm, slot)
        else:
            stage_A(i, *steps[s], kind, k_s, qT_s, sw, sy, sm, slot)

    B = lambda i, s, kind, slot, osl: stage_B(i, *steps[s], kind, vT_s, oT_s, sw, sy, sm, slot, osl)

    def yp(t0, c):
        t = t0 + c
        ypost(YT, u_s, Dv, b_s, t >> 4, (t & 15) >> 1, c % 2)

    A(0, 0, 0, 0)
    for s in range(8):
        if s % 4 == 0:
            yp(z, s // 4)
        if s < 7:
            A(0, s + 1, 0, (s + 1) % 2)
        else:
            A(1, 0, 1, 0)
        B(0, s, 0, s % 2, 0)
    for s in range(8):
        if s % 4 == 0:
            yp(z + 2, s // 4)
        if s < 7:
            A(1, s + 1, 1, (s + 1) % 2)
        else:
            A(2, 0, 2, 0)
        B(1, s, 1, s % 2, 1)
        if s == 1:
            outproj(oT_s, 0, wot_s, a_s, 0)

    def att_pair(i0, t0, last):
        for e in range(2):
            i = i0 + e
            for s in range(8):
                if t0 is not None and s < 5:
                    yp(t0, 5 * e + s)
                if s < 7:
                    A(i, s + 1, 2, (s + 1) % 2)
                elif not (last and e == 1):
                    A(i + 1, 0, 2, 0)
                B(i, s, 2, s % 2, e)
                if s == 1:
                    outproj(oT_s, 1 - e, wot_s, a_s, i - 1)

    start = lambda cps: [c.start() for c in cps]

    start(a_copies(0, 1))

    @pl.loop(0, 3)
    def _(it):
        i0 = 2 + 4 * it
        att_pair(i0, 4 + 20 * it, False)
        att_pair(i0 + 2, 14 + 20 * it, False)
        start(a_copies(i0 - 1, 4) + [b_copy(it)])

        @pl.when(it == 2)
        def _():
            b_copy(3).start()

    @block
    def _(z):
        att_pair(z + 14, None, True)
        start(a_copies(13, 2))

    outproj(oT_s, 1, wot_s, a_s, z + 15)
    start(a_copies(15, 1))
    for g in range(4):
        b_copy(g).wait()
    wait(a_copies(0, 1) + a_copies(1, 4) + a_copies(5, 4) + a_copies(9, 4) + a_copies(13, 2) + a_copies(15, 1))


def _scratch():
    T = lambda r: pltpu.VMEM((r, 128), F32)
    V = pltpu.VMEM
    s = [V((4, SEQ, 128), BF16), V((12, DM, 128), BF16), V((4, DM, 128), BF16), V((4, SEQ, 128), BF16)]
    s += [V((DM, 128), BF16)] * 6 + [V((DM,), BF16)] * 2
    s += [V((4, SEQ, 128), BF16), V((4, SEQ, 128), BF16), pltpu.SemaphoreType.DMA((13,))]
    s += [V((4, 1024, 128), BF16), V((4, DM, 128), BF16), V((4, SEQ, 128), BF16), V((16, DM, 128), BF16), V((16, DM, 128), BF16),
          V((2, DM, 128), BF16), V((2, 4, 128, 128), F32), V((2, 4, 128, 128), F32), V((2, 4, 8, 128), F32),
          T(8)]
    s += [T(512), T(512 * VP), T(512 * VP)] + [T(512)] * 11
    s += [V((256 * UP, 128), I32), V((256 * 128, 128), I32),
          V((256 * SPB, 128), BF16), V((256 * SPB, 128), BF16),
          V((256 * HP, 128), I32), V((256 * HP, 128), I32),
          V((8, 64, 128), F32), V((8, 64, 128), F32), V((256 * YP, 128), BF16)]
    return s


@jax.jit
def pallas_concat_heads__sliding_block__ssm_conv_s4__prompt_kernel(
    A_x: jax.Array,
    A_wqkv: jax.Array,
    A_wo: jax.Array,
    B_u: jax.Array,
    B_A_re: jax.Array,
    B_A_im: jax.Array,
    B_B_re: jax.Array,
    B_B_im: jax.Array,
    B_C_re: jax.Array,
    B_C_im: jax.Array,
    B_log_dt: jax.Array,
    B_Dskip: jax.Array,
):
    hbm = pl.BlockSpec(memory_space=pl.ANY)
    return pl.pallas_call(
        kernel_body,
        grid=(1,),
        in_specs=[hbm] * 12,
        out_specs=hbm,
        out_shape=jax.ShapeDtypeStruct((1, SEQ, 2 * DM), BF16),
        scratch_shapes=_scratch(),
        compiler_params=pltpu.CompilerParams(vmem_limit_bytes=110 * 1024 * 1024),
    )(A_x, A_wqkv, A_wo, B_u, B_A_re, B_A_im, B_B_re, B_B_im, B_C_re, B_C_im, B_log_dt, B_Dskip)
```
